```python
import os as _os
_os.environ.setdefault("JAX_PLATFORMS", "cpu")
import jax
import jax.numpy as jnp

def _softmax(x, axis=-1):
    return jax.nn.softmax(x, axis=axis)
def _gelu(x):
    return jax.nn.gelu(x, approximate=True)
def _silu(x):
    return jax.nn.silu(x)
def _sigmoid(x):
    return jax.nn.sigmoid(x)
def _layernorm(x, axis=-1, eps=1e-5):
    m = jnp.mean(x, axis=axis, keepdims=True)
    v = jnp.var(x, axis=axis, keepdims=True)
    return (x - m) / jnp.sqrt(v + eps)
def _scatter_add(tgt, idx, src, axis=0):
    return tgt.at[idx].add(src)
def _segment_sum(src, seg, n):
    return jax.ops.segment_sum(src, seg, n)
class _Rng:
    def __init__(self, key):
        self._k = key
    def _next(self):
        self._k, sub = jax.random.split(self._k)
        return sub
    def normal(self, shape):
        return jax.random.normal(self._next(), shape, dtype=jnp.bfloat16)
    def randint(self, lo, hi, shape):
        return jax.random.randint(self._next(), shape, lo, hi, dtype=jnp.int32)
    def uniform(self, shape, lo=0.0, hi=1.0):
        return jax.random.uniform(self._next(), shape, jnp.bfloat16, lo, hi)
    def permutation(self, n):
        return jax.random.permutation(self._next(), n)


kernel_name = 'recurrent_scan__linear_attn_block__geglu_ffn__prompt'

def setup_inputs():
    _rng = _Rng(jax.random.key(int.from_bytes(__import__("os").urandom(4), "little")))
    _w = (lambda a: (lambda t: t.astype(jnp.bfloat16) if jnp.issubdtype(t.dtype, jnp.floating) else t)(jnp.asarray(a)))
    def _A_setup():
        B, S, D = 1, 2048, 512
        return {
            "x": _w((lambda *s: _rng.normal(s) * 0.05)(B, S, D)),
            "wqkv": _w((lambda *s: _rng.normal(s) * 0.05)(D, 3 * D)),
            "wo": _w((lambda *s: _rng.normal(s) * 0.05)(D, D)),
        }
    _A_in = _A_setup()

    def _B_setup():
        B, S, D, F = 1, 2048, 512, 1792
        return {
            "x": _w((lambda *s: _rng.normal(s) * 0.05)(B, S, D)),
            "w_gate": _w((lambda *s: _rng.normal(s) * 0.05)(D, F)),
            "w_up": _w((lambda *s: _rng.normal(s) * 0.05)(D, F)),
            "w_down": _w((lambda *s: _rng.normal(s) * 0.05)(F, D)),
        }
    _B_in = _B_setup()

    return {
        "A_x": _A_in["x"],
        "A_wqkv": _A_in["wqkv"],
        "A_wo": _A_in["wo"],
        "B_x": _B_in["x"],
        "B_w_gate": _B_in["w_gate"],
        "B_w_up": _B_in["w_up"],
        "B_w_down": _B_in["w_down"],
    }

def reference(A_x, A_wqkv, A_wo, B_x, B_w_gate, B_w_up, B_w_down):
    def _A_ref(x, wqkv, wo):
        B, S, D = x.shape
        H = 32; Dh = D // H
        qkv = (lambda x, *d: x.transpose(*d))((x @ wqkv).reshape(B, S, 3, H, Dh), 2, 0, 3, 1, 4)
        q, k, v = qkv[0], qkv[1], qkv[2]
        phi = lambda t: jnp.where(t > 0, t + 1, jnp.exp(t)) + 1e-6
        pq, pk = phi(q), phi(k)
        kv = jnp.einsum("bhsd,bhse->bhde", pk, v)
        z = jnp.einsum("bhsd->bhd", pk)
        num = jnp.einsum("bhqd,bhde->bhqe", pq, kv)
        den = jnp.einsum("bhqd,bhd->bhq", pq, z)[..., None] + 1e-6
        o = num / den
        return (lambda x, *d: x.transpose(*d))(o, 0, 2, 1, 3).reshape(B, S, D) @ wo

    def _B_ref(x, w_gate, w_up, w_down):
        return (_gelu(x @ w_gate) * (x @ w_up)) @ w_down

    x = A_x
    xn = _layernorm(x, axis=-1)
    s = _A_ref(xn, A_wqkv, A_wo)
    g = _silu(_B_ref(xn, B_w_gate, B_w_up, B_w_down))
    return x + s * g
```

```python
import jax
import jax.numpy as jnp
from jax import lax
import jax.experimental.pallas as pl
import jax.experimental.pallas.tpu as pltpu

S, D, F = 2048, 512, 1792
H = 32
DH = D // H
G = 128
NG = D // G
HP = DH // 2
f32 = jnp.float32
bf16 = jnp.bfloat16
u32 = jnp.uint32


def _phi(t):
    return jnp.where(t > 0, t + 1.0, jnp.exp(t)) + 1e-6


def _gelu(x):
    c = 0.7978845608028654
    return 0.5 * x * (1.0 + jnp.tanh(c * (x + 0.044715 * (x * x * x))))


def _silu(d):
    hd = 0.5 * d
    return hd * (1.0 + jnp.tanh(hd))


def _dot(a, b):
    return jnp.dot(a, b, preferred_element_type=f32)


def _dot_nt(a, b):
    return lax.dot_general(a, b, (((1,), (1,)), ((), ())), preferred_element_type=f32)


def make(TM=256, CH="256-768-1024", T1=256, UNROLL=2, NOCHK=1, OSPLIT=4):
    NT = S // TM
    CHS = [int(c) for c in str(CH).split('-')]
    assert sum(CHS) == S
    OFF = [sum(CHS[:i]) for i in range(len(CHS))]
    NC = len(CHS)

    def kernel(x_hbm, wqkv_hbm, wo_hbm, wg_hbm, wu_hbm, wd_hbm, out_hbm,
               x_v, xn_v, wq_v, wk_v, wv_v, wo_v, wg_v, wu_v, wd_v, out_v,
               a_acc, z_acc, m_v, wqt_u, wkt_u, pk0_u, zrow_v, sem, osem):
        def xcopy(i):
            return pltpu.make_async_copy(x_hbm.at[pl.ds(OFF[i], CHS[i])], x_v.at[pl.ds(OFF[i], CHS[i])], sem.at[7 + i])
        wk_cp = pltpu.make_async_copy(wqkv_hbm.at[:, pl.ds(D, D)], wk_v, sem.at[0])
        wq_cp = pltpu.make_async_copy(wqkv_hbm.at[:, pl.ds(0, D)], wq_v, sem.at[1])
        wv_cp = pltpu.make_async_copy(wqkv_hbm.at[:, pl.ds(2 * D, D)], wv_v, sem.at[2])
        wo_cp = pltpu.make_async_copy(wo_hbm, wo_v, sem.at[3])
        wg_cp = pltpu.make_async_copy(wg_hbm, wg_v, sem.at[4])
        wu_cp = pltpu.make_async_copy(wu_hbm, wu_v, sem.at[5])
        wd_cp = pltpu.make_async_copy(wd_hbm, wd_v, sem.at[6])

        def store_t(dst_u, w):
            for c in range(dst_u.shape[0]):
                dst_u[c] = pltpu.bitcast(w[c * G:(c + 1) * G, :].T, u32)

        def load_perm(src_u):
            rows = []
            for dp in range(HP):
                blk = [src_u[c, pl.ds(dp, H, stride=HP), :] for c in range(src_u.shape[0])]
                blk = blk[0] if len(blk) == 1 else jnp.concatenate(blk, axis=1)
                rows.append(blk)
            return pltpu.bitcast(jnp.concatenate(rows, axis=0), bf16)

        def ln(o, t):
            r = pl.ds(o, t)
            x = x_v[r, :].astype(f32)
            m = jnp.mean(x, axis=-1, keepdims=True)
            xc = x - m
            v = jnp.mean(xc * xc, axis=-1, keepdims=True)
            xn_v[r, :] = (xc * lax.rsqrt(v + 1e-5)).astype(bf16)

        def kstage(o, t):
            pkt = _phi(_dot_nt(load_perm(wkt_u), xn_v[pl.ds(o, t), :]))
            zp = pkt[:, 0:128]
            for j in range(1, t // 128):
                zp = zp + pkt[:, j * 128:(j + 1) * 128]
            z_acc[...] += zp
            return pkt.astype(bf16)

        def astage(pktb, o, t):
            a = _dot(pktb, xn_v[pl.ds(o, t), :])
            if o == 0:
                a_acc[...] = a
            else:
                a_acc[...] += a

        def qstage(xn):
            pq = _phi(_dot_nt(xn, load_perm(wqt_u)))
            t = pq * zrow_v[0:1, :]
            t4 = (t[:, 0:G] + t[:, G:2 * G]) + (t[:, 2 * G:3 * G] + t[:, 3 * G:4 * G])
            u = t4 + pltpu.roll(t4, 64, 1)
            even = (lax.broadcasted_iota(jnp.int32, u.shape, 1) & 1) == 0
            den = u + jnp.where(even, pltpu.roll(u, G - 1, 1), pltpu.roll(u, 1, 1)) + 1e-6
            inv = pl.reciprocal(den, approx=True)
            return jnp.concatenate([pq[:, g * G:(g + 1) * G] * inv for g in range(NG)], axis=1).astype(bf16)

        xcopy(0).start()
        wk_cp.start()
        for i in range(1, NC):
            xcopy(i).start()
        for cp in (wq_cp, wv_cp, wo_cp, wg_cp, wu_cp, wd_cp):
            cp.start()

        xcopy(0).wait()
        for o in range(0, CHS[0], T1):
            ln(o, min(T1, CHS[0] - o))
        wk_cp.wait()
        store_t(pk0_u, _phi(_dot(xn_v[0:128, :], wk_v[...])).astype(bf16))
        store_t(wkt_u, wk_v)
        pk0t = load_perm(pk0_u)
        z_acc[...] = pk0t.astype(f32)
        pend = (pk0t, 0, 128)
        subs = [(128, CHS[0] - 128)] if CHS[0] > 128 else []
        for i in range(NC):
            if i > 0:
                xcopy(i).wait()
                if i == NC - 1:
                    wq_cp.wait()
                    wv_cp.wait()
                    wo_cp.wait()
                    store_t(wqt_u, wq_v)
                subs = [(o, min(T1, OFF[i] + CHS[i] - o)) for o in range(OFF[i], OFF[i] + CHS[i], T1)]
            for (o, t) in subs:
                if i > 0:
                    astage(*pend)
                    ln(o, t)
                    pend = (kstage(o, t), o, t)
                else:
                    nxt = (kstage(o, t), o, t)
                    astage(*pend)
                    pend = nxt
        astage(*pend)

        zrow_v[...] = jnp.broadcast_to(jnp.sum(z_acc[...].T, axis=0, keepdims=True), zrow_v.shape)

        ri = (lax.broadcasted_iota(jnp.int32, (G, G), 0) % DH) // 2
        ci = lax.broadcasted_iota(jnp.int32, (G, G), 1) // DH
        mask = ri == ci
        for g in range(NG):
            sl = slice(g * G, (g + 1) * G)
            ag = jnp.concatenate([a_acc[pl.ds(dp * 2 * H + DH * g, DH), :] for dp in range(HP)], axis=0)
            kv = _dot(ag.astype(bf16), wv_v[:, sl])
            kv = jnp.where(mask, kv, 0.0).astype(bf16)
            mg = _dot(kv, wo_v[sl, :]).astype(bf16)
            for dp in range(HP):
                m_v[pl.ds(dp * 2 * H + DH * g, DH), :] = mg[dp * DH:(dp + 1) * DH, :]

        wg_cp.wait()
        wu_cp.wait()
        wd_cp.wait()

        def phase2(i, c):
            r = pl.ds(i * TM if isinstance(i, int) else pl.multiple_of(i * TM, TM), TM)
            xn = xn_v[r, :]
            rr = qstage(xn)
            gate = _dot(xn, wg_v[...])
            up = _dot(xn, wu_v[...])
            h = (_gelu(gate) * up).astype(bf16)
            d = _dot(h, wd_v[...])
            gt = _silu(d)
            w = D // OSPLIT
            for j in range(OSPLIT):
                cs = pl.ds(j * w, w)
                s = _dot(rr, m_v[:, cs])
                out_v[r, cs] = (x_v[r, cs].astype(f32) + s * gt[:, j * w:(j + 1) * w]).astype(bf16)
                pltpu.make_async_copy(out_v.at[r, cs], out_hbm.at[r, cs], osem.at[0]).start()
            return c

        lax.fori_loop(0, NT, phase2, 0, unroll=UNROLL)
        pltpu.make_async_copy(out_v, out_hbm, osem.at[0]).wait()

    @jax.jit
    def fn(A_x, A_wqkv, A_wo, B_x, B_w_gate, B_w_up, B_w_down):
        x = A_x.reshape(S, D)
        anyspec = pl.BlockSpec(memory_space=pl.ANY)
        out = pl.pallas_call(
            kernel,
            out_shape=jax.ShapeDtypeStruct((S, D), bf16),
            in_specs=[anyspec] * 6,
            out_specs=anyspec,
            scratch_shapes=[
                pltpu.VMEM((S, D), bf16),
                pltpu.VMEM((S, D), bf16),
                pltpu.VMEM((D, D), bf16),
                pltpu.VMEM((D, D), bf16),
                pltpu.VMEM((D, D), bf16),
                pltpu.VMEM((D, D), bf16),
                pltpu.VMEM((D, F), bf16),
                pltpu.VMEM((D, F), bf16),
                pltpu.VMEM((F, D), bf16),
                pltpu.VMEM((S, D), bf16),
                pltpu.VMEM((D, D), f32),
                pltpu.VMEM((D, 128), f32),
                pltpu.VMEM((D, D), bf16),
                pltpu.VMEM((NG, D // 2, G), u32),
                pltpu.VMEM((NG, D // 2, G), u32),
                pltpu.VMEM((1, D // 2, G), u32),
                pltpu.VMEM((8, D), f32),
                pltpu.SemaphoreType.DMA((7 + NC,)),
                pltpu.SemaphoreType.DMA((1,)),
            ],
            compiler_params=pltpu.CompilerParams(vmem_limit_bytes=100 * 1024 * 1024,
                                                 disable_bounds_checks=bool(NOCHK), disable_semaphore_checks=bool(NOCHK)),
        )(x, A_wqkv, A_wo, B_w_gate, B_w_up, B_w_down)
        return out.reshape(1, S, D)

    return fn


pallas_recurrent_scan__linear_attn_block__geglu_ffn__prompt_kernel = make()
```

```python
import jax
import jax.numpy as jnp
from jax import lax
import jax.experimental.pallas as pl
import jax.experimental.pallas.tpu as pltpu

S, D, F = 2048, 512, 1792
H = 32
DH = D // H
G = 128
NG = D // G
HP = DH // 2
HG = G // DH
HD = D // 2

X_CHUNKS = (256, 128, 896, 768)
X_OFFS = tuple(sum(X_CHUNKS[:i]) for i in range(len(X_CHUNKS)))
T1 = 256
TILES = (256, 512, 256)
RB = sum(TILES)
NIT = S // RB
LAST_SPLIT = 4

f32 = jnp.float32
bf16 = jnp.bfloat16
u32 = jnp.uint32


def _phi(t):
    return jnp.where(t > 0, t + 1.0, jnp.exp(t)) + 1e-6


def _gelu(x):
    c = 0.7978845608028654
    return 0.5 * x * (1.0 + jnp.tanh(c * (x + 0.044715 * (x * x * x))))


def _silu(d):
    hd = 0.5 * d
    return hd * (1.0 + jnp.tanh(hd))


def _dot(a, b):
    return jnp.dot(a, b, preferred_element_type=f32)


def _dot_nt(a, b):
    return lax.dot_general(a, b, (((1,), (1,)), ((), ())), preferred_element_type=f32)


def _lanesum(p):
    zp = p[:, 0:G]
    for j in range(1, p.shape[1] // G):
        zp = zp + p[:, j * G:(j + 1) * G]
    return zp


def _kernel(x_hbm, wqkv_hbm, wo_hbm, wg_hbm, wu_hbm, wd_hbm, out_hbm,
            x_v, xn_u, wq_v, wk_v, wv_v, wo_v, wg_v, wu_v, wd_v, out_v,
            a_acc, z_acc, m_v, wqt_u, wkt_u, pk0_u, zrow_v, pq_v, sem, osem, one):
    nc = len(X_CHUNKS)
    xa = X_CHUNKS[0]

    def xcopy(i):
        rows = pl.ds(X_OFFS[i], X_CHUNKS[i])
        return pltpu.make_async_copy(x_hbm.at[rows], x_v.at[rows], sem.at[8 + i])

    wk_cp = [pltpu.make_async_copy(wqkv_hbm.at[:, pl.ds(D + hh * HD, HD)], wk_v.at[hh], sem.at[7 * hh])
             for hh in range(2)]
    wq_cp = pltpu.make_async_copy(wqkv_hbm.at[:, pl.ds(0, D)], wq_v, sem.at[1])
    wv_cp = pltpu.make_async_copy(wqkv_hbm.at[:, pl.ds(2 * D, D)], wv_v, sem.at[2])
    wo_cp = pltpu.make_async_copy(wo_hbm, wo_v, sem.at[3])
    wg_cp = pltpu.make_async_copy(wg_hbm, wg_v, sem.at[4])
    wu_cp = pltpu.make_async_copy(wu_hbm, wu_v, sem.at[5])
    wd_cp = pltpu.make_async_copy(wd_hbm, wd_v, sem.at[6])

    def store_t(dst_u, w, p0=0):
        n = w.shape[1] // 2
        for c in range(dst_u.shape[0]):
            dst_u[c, pl.ds(p0, n), :] = pltpu.bitcast(w[c * G:(c + 1) * G, :].T, u32)

    def load_rows(src_u, blocks):
        rows = []
        for p0, nh in blocks:
            blk = [src_u[c, pl.ds(p0, nh, stride=HP), :] for c in range(src_u.shape[0])]
            rows.append(jnp.concatenate(blk, axis=1))
        return pltpu.bitcast(jnp.concatenate(rows, axis=0), bf16)

    def load_qorder(src_u):
        return load_rows(src_u, [(dp, H) for dp in range(HP)])

    def load_korder(src_u, groups=range(NG)):
        return load_rows(src_u, [(g * HG * HP + dp, HG) for g in groups for dp in range(HP)])

    def ln(o, t):
        x = x_v[pl.ds(o, t), :].astype(f32)
        m = jnp.mean(x, axis=-1, keepdims=True)
        xc = x - m
        v = jnp.mean(xc * xc, axis=-1, keepdims=True)
        xn = (xc * lax.rsqrt(v + 1e-5)).astype(bf16)
        xn_u[pl.ds(o // 2, t // 2), :] = pltpu.bitcast(xn, u32)
        return xn

    def load_xn(pair0, t):
        return pltpu.bitcast(xn_u[pl.ds(pair0, t // 2), :], bf16)

    def kstage(xn):
        pkt = _phi(_dot_nt(load_korder(wkt_u), xn))
        z_acc[...] += _lanesum(pkt)
        return pkt.astype(bf16)

    def astage(pktb, o, t):
        a_acc[...] += _dot(pktb, load_xn(o // 2, t))

    def a0half(hh):
        pk = load_korder(pk0_u, (2 * hh, 2 * hh + 1))
        rs = pl.ds(hh * HD, HD)
        a_acc[rs, :] = _dot(pk, load_xn(0, xa))
        z_acc[rs, :] = _lanesum(pk.astype(f32))

    def qproj(xn):
        return _phi(_dot_nt(xn, load_qorder(wqt_u)))

    def qnorm(pq):
        t4 = _lanesum(pq * zrow_v[0:1, :])
        u = t4 + pltpu.roll(t4, 64, 1)
        even = (lax.broadcasted_iota(jnp.int32, u.shape, 1) & 1) == 0
        den = u + jnp.where(even, pltpu.roll(u, G - 1, 1), pltpu.roll(u, 1, 1)) + 1e-6
        inv = 1.0 / den
        return jnp.concatenate([pq[:, g * G:(g + 1) * G] * inv for g in range(NG)], axis=1).astype(bf16)

    def tile(it, o, t, first, last):
        base = it * RB + o
        r = pl.ds(pl.multiple_of(base, 64), t)
        xn = load_xn(pl.multiple_of(it * (RB // 2) + o // 2, 32), t)
        gate = _dot(xn, wg_v[...])
        up = _dot(xn, wu_v[...])
        h = (_gelu(gate) * up).astype(bf16)
        rr = qnorm(pq_v[it] if first else qproj(xn))
        gt = _silu(_dot(h, wd_v[...]))
        for j in range(NG):
            cs = pl.ds(j * G, G)
            s = _dot(rr, m_v[:, cs])
            y = (x_v[r, cs].astype(f32) + s * gt[:, j * G:(j + 1) * G]).astype(bf16)
            parts = LAST_SPLIT if (last and j == NG - 1) else 1
            tp = t // parts
            for p in range(parts):
                rp = pl.ds(pl.multiple_of(base + p * tp, 16), tp)
                out_v[rp, cs] = y[p * tp:(p + 1) * tp, :]
                pltpu.make_async_copy(out_v.at[rp, cs], out_hbm.at[rp, cs], osem.at[0]).start()

    def phase2(it, carry):
        o = 0
        for k, t in enumerate(TILES):
            tile(it, o, t, k == 0, k == len(TILES) - 1)
            o += t
        return carry

    def main(_, carry):
        xcopy(0).wait()
        ln(0, xa)
        wk_cp[0].wait()
        pka = _phi(_dot(load_xn(0, xa), wk_v[0])).astype(bf16)
        store_t(wkt_u, wk_v.at[0], 0)
        xcopy(1).wait()
        wk_cp[1].wait()
        store_t(pk0_u, pka, 0)
        store_t(pk0_u, _phi(_dot(load_xn(0, xa), wk_v[1])).astype(bf16), HD // 2)
        store_t(wkt_u, wk_v.at[1], HD // 2)
        xnb = ln(X_OFFS[1], X_CHUNKS[1])
        a0half(0)
        pkt = _phi(_dot_nt(load_korder(wkt_u), xnb))
        a0half(1)
        z_acc[...] += _lanesum(pkt)
        pend = (pkt.astype(bf16), X_OFFS[1], X_CHUNKS[1])
        for i in range(2, nc):
            xcopy(i).wait()
            if i == nc - 1:
                wq_cp.wait()
                wv_cp.wait()
                wo_cp.wait()
                store_t(wqt_u, wq_v)
            lo, n = X_OFFS[i], X_CHUNKS[i]
            rem = n % T1
            for o, t in ([(lo, rem)] if rem else []) + [(o, T1) for o in range(lo + rem, lo + n, T1)]:
                astage(*pend)
                pend = (kstage(ln(o, t)), o, t)
        astage(*pend)

        zq = jnp.concatenate([z_acc[pl.ds(g * G + dp * DH, DH), :] for dp in range(HP) for g in range(NG)], axis=0)
        zrow_v[...] = jnp.broadcast_to(jnp.sum(zq.T, axis=0, keepdims=True), zrow_v.shape)

        row_head = (lax.broadcasted_iota(jnp.int32, (G, G), 0) % DH) // 2
        col_head = lax.broadcasted_iota(jnp.int32, (G, G), 1) // DH
        same_head = row_head == col_head
        kvs = []
        for g in range(NG):
            sl = slice(g * G, (g + 1) * G)
            kv = _dot(a_acc[sl, :].astype(bf16), wv_v[:, sl])
            kvs.append(jnp.where(same_head, kv, 0.0).astype(bf16))
        for it in range(NIT):
            pq_v[it] = qproj(load_xn(it * RB // 2, TILES[0]))
        for g in range(NG):
            mg = _dot(kvs[g], wo_v[g * G:(g + 1) * G, :]).astype(bf16)
            for dp in range(HP):
                m_v[pl.ds(dp * 2 * H + DH * g, DH), :] = mg[dp * DH:(dp + 1) * DH, :]

        wg_cp.wait()
        wu_cp.wait()
        wd_cp.wait()
        lax.fori_loop(0, NIT, phase2, 0)
        return carry

    one[0] = 1
    xcopy(0).start()
    wk_cp[0].start()
    xcopy(1).start()
    wk_cp[1].start()
    for i in range(2, nc):
        xcopy(i).start()
    for cp in (wq_cp, wv_cp, wo_cp, wg_cp, wu_cp, wd_cp):
        cp.start()
    lax.fori_loop(0, one[0], main, 0)
    pltpu.make_async_copy(out_v, out_hbm, osem.at[0]).wait()


@jax.jit
def pallas_recurrent_scan__linear_attn_block__geglu_ffn__prompt_kernel(
    A_x: jax.Array,
    A_wqkv: jax.Array,
    A_wo: jax.Array,
    B_x: jax.Array,
    B_w_gate: jax.Array,
    B_w_up: jax.Array,
    B_w_down: jax.Array,
):
    del B_x
    hbm = pl.BlockSpec(memory_space=pl.ANY)
    pairs = D // 2 + HP
    out = pl.pallas_call(
        _kernel,
        out_shape=jax.ShapeDtypeStruct((S, D), bf16),
        in_specs=[hbm] * 6,
        out_specs=hbm,
        scratch_shapes=[
            pltpu.VMEM((S, D), bf16),
            pltpu.VMEM((S // 2, D), u32),
            pltpu.VMEM((D, D), bf16),
            pltpu.VMEM((2, D, HD), bf16),
            pltpu.VMEM((D, D), bf16),
            pltpu.VMEM((D, D), bf16),
            pltpu.VMEM((D, F), bf16),
            pltpu.VMEM((D, F), bf16),
            pltpu.VMEM((F, D), bf16),
            pltpu.VMEM((S, D), bf16),
            pltpu.VMEM((D, D), f32),
            pltpu.VMEM((D, G), f32),
            pltpu.VMEM((D, D), bf16),
            pltpu.VMEM((NG, pairs, G), u32),
            pltpu.VMEM((NG, pairs, G), u32),
            pltpu.VMEM((X_CHUNKS[0] // G, pairs, G), u32),
            pltpu.VMEM((8, D), f32),
            pltpu.VMEM((NIT, TILES[0], D), f32),
            pltpu.SemaphoreType.DMA((8 + len(X_CHUNKS),)),
            pltpu.SemaphoreType.DMA((1,)),
            pltpu.SMEM((1,), jnp.int32),
        ],
        compiler_params=pltpu.CompilerParams(
            vmem_limit_bytes=100 * 1024 * 1024,
            disable_bounds_checks=True,
            disable_semaphore_checks=True,
        ),
    )(A_x.reshape(S, D), A_wqkv, A_wo, B_w_gate, B_w_up, B_w_down)
    return out.reshape(1, S, D)
```

```python
import contextlib
import jax
import jax.numpy as jnp
from jax import lax
import jax.experimental.pallas as pl
import jax.experimental.pallas.tpu as pltpu

S, D, F = 2048, 512, 1792
H = 32
DH = D // H
G = 128
NG = D // G
HP = DH // 2
HG = G // DH
HD = D // 2
HF = F // 2
HS = S // 2
f32 = jnp.float32
bf16 = jnp.bfloat16
u32 = jnp.uint32


def _phi(t):
    return jnp.where(t > 0, t + 1.0, jnp.exp(t)) + 1e-6


def _gelu(x):
    c = 0.7978845608028654
    return 0.5 * x * (1.0 + jnp.tanh(c * (x + 0.044715 * (x * x * x))))


def _silu(d):
    hd = 0.5 * d
    return hd * (1.0 + jnp.tanh(hd))


def _dot(a, b):
    return jnp.dot(a, b, preferred_element_type=f32)


def _dot_nt(a, b):
    return lax.dot_general(a, b, (((1,), (1,)), ((), ())), preferred_element_type=f32)


def _lanesum(p):
    zp = p[:, 0:G]
    for j in range(1, p.shape[1] // G):
        zp = zp + p[:, j * G:(j + 1) * G]
    return zp


def _lhs7(a11, a12, a21, a22):
    c11, c12, c21, c22 = [x.astype(f32) for x in (a11, a12, a21, a22)]
    return [x.astype(bf16) for x in (c11 + c22, c21 + c22, a11, a22, c11 + c12, c21 - c11, c12 - c22)]


def _rhs7(b11, b12, b21, b22):
    c11, c12, c21, c22 = [x.astype(f32) for x in (b11, b12, b21, b22)]
    return [x.astype(bf16) for x in (c11 + c22, b11, c12 - c22, c21 - c11, b22, c11 + c12, c21 + c22)]


def _strassen(prod):
    m5 = prod(4)
    m3 = prod(2)
    c12 = m3 + m5
    m2 = prod(1)
    m4 = prod(3)
    c21 = m2 + m4
    m1 = prod(0)
    c11 = prod(6) + (m1 + (m4 - m5))
    c22 = prod(5) + (m1 + (m3 - m2))
    return c11, c12, c21, c22


def make(CH="128-128-128-768-896", T1=512, NOCHK=1, SC=0, LS=2, ASPLIT=2, NIT=2, PAD=16, QP=4, QAT="1-2-4-5", QPRE=1, SBS="128-128-128-64-64", DORD="2-4-5-1-3-0-6", QS=16):
    P = HS // NIT
    CHS = [int(c) // 2 for c in str(CH).split('-')]
    assert sum(CHS) == HS
    OFF = [sum(CHS[:i]) for i in range(len(CHS))]
    NC = len(CHS)
    B0 = G // 2
    assert CHS[0] == CHS[1] == B0
    T1H = T1 // 2
    QATS = [int(c) for c in str(QAT).split('-')]
    SB = [int(c) for c in str(SBS).split('-')]
    assert sum(SB) == P
    TQ = P // QP
    DO = [int(c) for c in DORD.split('-')]
    scope = (lambda n: jax.named_scope(n)) if SC else (lambda n: contextlib.nullcontext())

    def kernel(x_hbm, wqkv_hbm, wo_hbm, wg_hbm, wu_hbm, wd_hbm, out_hbm,
               x_v, xn_u, wq_v, wk_v, wv_v, wo_v, wg_v, wu_v, wd_v, out_v,
               a_acc, z_acc, rm_u, rq_u, pq_v, wqt_u, wkt_u, pk0_u, zrow_v, sem, osem, cnt):
        def xcopy(i):
            rows = pl.ds(OFF[i], CHS[i])
            return pltpu.make_async_copy(x_hbm.at[:, rows], x_v.at[:, rows], sem.at[8 + i])
        wk_cp = [pltpu.make_async_copy(wqkv_hbm.at[:, pl.ds(D + hh * HD, HD)], wk_v.at[hh], sem.at[7 * hh])
                 for hh in range(2)]
        wq_cp = pltpu.make_async_copy(wqkv_hbm.at[:, pl.ds(0, D)], wq_v, sem.at[1])
        wv_cp = pltpu.make_async_copy(wqkv_hbm.at[:, pl.ds(2 * D, D)], wv_v, sem.at[2])
        wo_cp = pltpu.make_async_copy(wo_hbm, wo_v, sem.at[3])
        wg_cp = pltpu.make_async_copy(wg_hbm, wg_v, sem.at[4])
        wu_cp = pltpu.make_async_copy(wu_hbm, wu_v, sem.at[5])
        wd_cp = pltpu.make_async_copy(wd_hbm, wd_v, sem.at[6])

        def store_t(dst_u, w, p0=0):
            n = w.shape[1] // 2
            for c in range(dst_u.shape[0]):
                dst_u[c, pl.ds(p0, n), :] = pltpu.bitcast(w[c * G:(c + 1) * G, :].T, u32)

        def load_rows(src_u, blocks, cs=None):
            rows = []
            for p0, nh in blocks:
                blk = [src_u[c, pl.ds(p0, nh, stride=HP), :] for c in (cs or range(src_u.shape[0]))]
                rows.append(blk[0] if len(blk) == 1 else jnp.concatenate(blk, axis=1))
            return pltpu.bitcast(jnp.concatenate(rows, axis=0), bf16)

        def load_qorder(src_u):
            return load_rows(src_u, [(dp, H) for dp in range(HP)])

        def load_korder(src_u, groups=range(NG), cs=None):
            return load_rows(src_u, [(g * HG * HP + dp, HG) for g in groups for dp in range(HP)], cs)

        def raw_x(o, t):
            return jnp.concatenate([x_v[0, pl.ds(o, t), :], x_v[1, pl.ds(o, t), :]], axis=0)

        def ln(o, t, stats=False):
            x = raw_x(o, t).astype(f32)
            m = jnp.mean(x, axis=-1, keepdims=True)
            xc = x - m
            v = jnp.mean(xc * xc, axis=-1, keepdims=True)
            rstd = lax.rsqrt(v + 1e-5)
            xn = (xc * rstd).astype(bf16)
            for hf in range(2):
                xn_u[hf, pl.ds(o // 2, t // 2), :] = pltpu.bitcast(xn[hf * t:(hf + 1) * t], u32)
            return (m, rstd) if stats else xn

        def load_blk(hf, pair0, t, cols=slice(None)):
            return pltpu.bitcast(xn_u[hf, pl.ds(pair0, t // 2), cols], bf16)

        def load_xn(o, t, half=None):
            cols = slice(None) if half is None else slice(half * HD, (half + 1) * HD)
            return jnp.concatenate([load_blk(0, o // 2, t, cols), load_blk(1, o // 2, t, cols)], axis=0)

        def kstage(xn):
            pkt = _phi(_dot_nt(load_korder(wkt_u), xn))
            z_acc[...] += _lanesum(pkt)
            return pkt.astype(bf16)

        def astage(pktb, o, t, half=None):
            cols = slice(None) if half is None else slice(half * HD, (half + 1) * HD)
            a_acc[:, cols] += _dot(pktb, load_xn(o, t, half))

        def qnorm(pq):
            t4 = _lanesum(pq * zrow_v[0:1, :])
            u = t4 + pltpu.roll(t4, 64, 1)
            even = (lax.broadcasted_iota(jnp.int32, u.shape, 1) & 1) == 0
            den = u + jnp.where(even, pltpu.roll(u, G - 1, 1), pltpu.roll(u, 1, 1)) + 1e-6
            return 1.0 / den

        def lhs_x(pair0, t):
            return _lhs7(*[load_blk(hf, pair0, t, slice(c0, c0 + HD)) for hf in range(2) for c0 in (0, HD)])

        def qproj(l7):
            q11, q12, q21, q22 = _strassen(lambda i: _dot(l7[i], pltpu.bitcast(rq_u[i], bf16)))
            return _phi(jnp.concatenate([q11, q12], axis=1)), _phi(jnp.concatenate([q21, q22], axis=1))

        cnt[0] = 1
        xcopy(0).start()
        wk_cp[0].start()
        xcopy(1).start()
        wk_cp[1].start()
        for i in range(2, NC):
            xcopy(i).start()
        for cp in (wq_cp, wv_cp, wo_cp, wg_cp, wu_cp, wd_cp):
            cp.start()

        def body(it, carry):
          with scope('iter'):
            base = pl.multiple_of(it * P, P)
            pair0 = pl.multiple_of(it * (P // 2), P // 2)
            lx = lhs_x(pair0, P)
            lrs = []

            def qfinish(pt, pb):
                parts = []
                for r0 in range(0, TQ, QS):
                    ps = [p[r0:r0 + QS] for p in (pt, pb)]
                    iv = [qnorm(p) for p in ps]
                    iv = [jnp.concatenate([v, v], axis=1) for v in iv]
                    parts.append(_lhs7(ps[0][:, :HD] * iv[0], ps[0][:, HD:] * iv[0],
                                       ps[1][:, :HD] * iv[1], ps[1][:, HD:] * iv[1]))
                lrs.append([jnp.concatenate([p[i] for p in parts], axis=0) for i in range(7)])

            if QPRE:
                qfinish(pq_v[it, 0], pq_v[it, 1])
            md = [None] * 7
            for n in range(HF // G):
                for _ in range(QATS.count(n)):
                    j = len(lrs)
                    if j < QP:
                        qfinish(*qproj([l[j * TQ:(j + 1) * TQ] for l in lx]))
                c1, c2 = pl.ds(n * G, G), pl.ds(HF + n * G, G)
                blocks = [jnp.concatenate([wg_v[pl.ds(k0, HD), c], wu_v[pl.ds(k0, HD), c]], axis=1)
                          for k0 in (0, HD) for c in (c1, c2)]
                r7 = _rhs7(*blocks)
                cs = _strassen(lambda i: _dot(lx[i], r7[i]))
                lh = _lhs7(*[_gelu(c[:, :G]) * c[:, G:] for c in cs])
                rd = _rhs7(*[wd_v[c, pl.ds(n0, HD)] for c in (c1, c2) for n0 in (0, HD)])
                for i in DO:
                    if i == DO[-1]:
                        d = jnp.concatenate([_dot(lh[i][:P // 2], rd[i]), _dot(lh[i][P // 2:], rd[i])], axis=0)
                    else:
                        d = _dot(lh[i], rd[i])
                    md[i] = d if md[i] is None else d + md[i]
            assert len(lrs) == QP
            gts = [_silu(d) for d in _strassen(lambda i: md[i])]
            lr = [jnp.concatenate([l[i] for l in lrs], axis=0) for i in range(7)]
            for b, ts in enumerate(SB):
                o = sum(SB[:b])
                rs = slice(o, o + ts)
                ss = _strassen(lambda i: _dot(lr[i][rs], pltpu.bitcast(rm_u[i], bf16)))
                for k in (1, 2, 0, 3):
                    half, cs = k // 2, pl.ds((k % 2) * HD, HD)
                    r0 = base + o
                    xr = x_v[half, pl.ds(pl.multiple_of(r0, 16), ts), cs]
                    y = (xr.astype(f32) + ss[k] * gts[k][rs]).astype(bf16)
                    parts = LS if (b == len(SB) - 1 and k == 3) else 1
                    tp = ts // parts
                    for p in range(parts):
                        rp = pl.ds(pl.multiple_of(r0 + p * tp, 16), tp)
                        out_v[half, rp, cs] = y[p * tp:(p + 1) * tp, :]
                        pltpu.make_async_copy(out_v.at[half, rp, cs], out_hbm.at[half, rp, cs], osem.at[0]).start()
          return carry

        def main(_, carry):
            with scope('w_x0'):
                xcopy(0).wait()
            ln(0, B0)
            with scope('w_wka'):
                wk_cp[0].wait()
            pk11 = _phi(_dot(load_xn(0, B0), wk_v[0])).astype(bf16)
            store_t(wkt_u, wk_v.at[0], 0)
            csum = jnp.sum(wk_v[0].astype(f32), axis=0, keepdims=True)
            with scope('w_x1'):
                xcopy(1).wait()
            y = _dot(raw_x(B0, B0), wk_v[0])
            m, rstd = ln(B0, B0, stats=True)
            pk21 = _phi((y - m * csum) * rstd).astype(bf16)
            pk0_u[0, pl.ds(0, HD // 2), :] = pltpu.bitcast(pk11.T, u32)
            ha, hb = pl.ds(0, HD), pl.ds(HD, HD)
            pk = load_korder(pk0_u, (0, 1), (0,))
            a_acc[ha, :] = _dot(pk, load_xn(0, B0))
            z_acc[ha, :] = pk.astype(f32)
            with scope('w_wkb'):
                wk_cp[1].wait()
                xcopy(2).wait()
            pk0_u[1, pl.ds(0, HD // 2), :] = pltpu.bitcast(pk21.T, u32)
            xn01 = jnp.concatenate([load_xn(0, B0), load_xn(B0, B0)], axis=0)
            store_t(pk0_u, _phi(_dot(xn01, wk_v[1])).astype(bf16), HD // 2)
            store_t(wkt_u, wk_v.at[1], HD // 2)
            xnb = ln(OFF[2], CHS[2])
            pk = load_korder(pk0_u, (0, 1), (1,))
            a_acc[ha, :] += _dot(pk, load_xn(B0, B0))
            z_acc[ha, :] += pk.astype(f32)
            pkt = _phi(_dot_nt(load_korder(wkt_u), xnb))
            pk = load_korder(pk0_u, (2, 3))
            a_acc[hb, :] = _dot(pk, xn01)
            z_acc[hb, :] = _lanesum(pk.astype(f32))
            z_acc[...] += _lanesum(pkt)
            pend = (pkt.astype(bf16), OFF[2], CHS[2])
            for i in range(3, NC):
                with scope('w_x%d' % i):
                    xcopy(i).wait()
                    if i == NC - 1:
                        wq_cp.wait()
                        wv_cp.wait()
                        wo_cp.wait()
                if i == NC - 1:
                    store_t(wqt_u, wq_v)
                    wqp = load_qorder(wqt_u).T
                    for k, op in enumerate(_rhs7(wqp[:HD, :HD], wqp[:HD, HD:], wqp[HD:, :HD], wqp[HD:, HD:])):
                        rq_u[k] = pltpu.bitcast(op, u32)
                rem = CHS[i] % T1H
                subs = ([(OFF[i], rem)] if rem else []) + [(o, T1H) for o in range(OFF[i] + rem, OFF[i] + CHS[i], T1H)]
                for (o, t) in subs:
                    astage(*pend)
                    pend = (kstage(ln(o, t)), o, t)
                if ASPLIT and i < NC - 1:
                    astage(*pend, 0)
                    pend = pend + (1,)
            astage(*pend)

            zq = jnp.concatenate([z_acc[pl.ds(g * G + dp * DH, DH), :] for dp in range(HP) for g in range(NG)], axis=0)
            zrow_v[...] = jnp.broadcast_to(jnp.sum(zq.T, axis=0, keepdims=True), zrow_v.shape)

            ri = (lax.broadcasted_iota(jnp.int32, (G, G), 0) % DH) // 2
            ci = lax.broadcasted_iota(jnp.int32, (G, G), 1) // DH
            mask = ri == ci
            kvs = []
            for g in range(NG):
                sl = slice(g * G, (g + 1) * G)
                kv = _dot(a_acc[sl, :].astype(bf16), wv_v[:, sl])
                kvs.append(jnp.where(mask, kv, 0.0).astype(bf16))
            def qpre(it):
                pt, pb = qproj(lhs_x(it * P // 2, TQ))
                pq_v[it, 0] = pt
                pq_v[it, 1] = pb

            if QPRE:
                for it in range(NIT - 1):
                    qpre(it)
            for g in range(NG):
                mg = _dot(kvs[g], wo_v[g * G:(g + 1) * G, :])
                hg = G // 2
                for k, op in enumerate(_rhs7(mg[:hg, :HD], mg[:hg, HD:], mg[hg:, :HD], mg[hg:, HD:])):
                    opu = pltpu.bitcast(op, u32)
                    for dp in range(HP // 2):
                        rm_u[k, pl.ds(dp * H + HP * g, HP), :] = opu[dp * HP:(dp + 1) * HP, :]

            if QPRE:
                qpre(NIT - 1)
            with scope('w_gud'):
                wg_cp.wait()
                wu_cp.wait()
                wd_cp.wait()
            lax.fori_loop(0, NIT, body, 0)
            return carry

        lax.fori_loop(0, cnt[0], main, 0)
        with scope('w_out'):
            pltpu.make_async_copy(out_v, out_hbm, osem.at[0]).wait()

    @jax.jit
    def fn(A_x, A_wqkv, A_wo, B_x, B_w_gate, B_w_up, B_w_down):
        x = A_x.reshape(2, HS, D)
        anyspec = pl.BlockSpec(memory_space=pl.ANY)
        out = pl.pallas_call(
            kernel,
            out_shape=jax.ShapeDtypeStruct((2, HS, D), bf16),
            in_specs=[anyspec] * 6,
            out_specs=anyspec,
            scratch_shapes=[
                pltpu.VMEM((2, HS, D), bf16),
                pltpu.VMEM((2, HS // 2, D), u32),
                pltpu.VMEM((D, D), bf16),
                pltpu.VMEM((2, D, HD), bf16),
                pltpu.VMEM((D, D), bf16),
                pltpu.VMEM((D, D), bf16),
                pltpu.VMEM((D, F), bf16),
                pltpu.VMEM((D, F), bf16),
                pltpu.VMEM((F, D), bf16),
                pltpu.VMEM((2, HS, D), bf16),
                pltpu.VMEM((D, D), f32),
                pltpu.VMEM((D, G), f32),
                pltpu.VMEM((7, HD // 2, HD), u32),
                pltpu.VMEM((7, HD // 2, HD), u32),
                pltpu.VMEM((NIT, 2, TQ, D), f32),
                pltpu.VMEM((NG, D // 2 + PAD, G), u32),
                pltpu.VMEM((NG, D // 2 + PAD, G), u32),
                pltpu.VMEM((2, D // 2 + PAD, G), u32),
                pltpu.VMEM((8, D), f32),
                pltpu.SemaphoreType.DMA((8 + NC,)),
                pltpu.SemaphoreType.DMA((1,)),
                pltpu.SMEM((1,), jnp.int32),
            ],
            compiler_params=pltpu.CompilerParams(vmem_limit_bytes=100 * 1024 * 1024,
                                                 disable_bounds_checks=bool(NOCHK), disable_semaphore_checks=bool(NOCHK)),
        )(x, A_wqkv, A_wo, B_w_gate, B_w_up, B_w_down)
        return out.reshape(1, S, D)

    return fn


pallas_recurrent_scan__linear_attn_block__geglu_ffn__prompt_kernel = make(QP=2,QAT='3')
```

```python
import jax
import jax.numpy as jnp
from jax import lax
import jax.experimental.pallas as pl
import jax.experimental.pallas.tpu as pltpu

S, D, F = 2048, 512, 1792
H = 32
DH = D // H
G = 128
NG = D // G
HP = DH // 2
HG = G // DH
HS, HD, HF = S // 2, D // 2, F // 2

X_CHUNKS = (64, 64, 64, 448, 384)
X_OFFS = tuple(sum(X_CHUNKS[:i]) for i in range(len(X_CHUNKS)))
B0 = X_CHUNKS[0]
R0 = 2 * G
NIT = 2
P = HS // NIT
TQ = P // 2
OUT_BLOCKS = (256, 128, 64, 64)
LAST_SPLIT = 2
A_ORDER = (2, 4, 3, 0, 6, 5, 1)
D_ORDER = (2, 5, 3, 0, 1, 4, 6)
X_AS_RHS = (0, 2, 6, 5, 3, 4, 1)

f32 = jnp.float32
bf16 = jnp.bfloat16
u32 = jnp.uint32


def _phi(t):
    return jnp.where(t > 0, t + 1.0, jnp.exp(t)) + 1e-6


def _geglu2(x, up):
    c = 0.7978845608028654
    return (x * up) * (1.0 + jnp.tanh(x * (c + (c * 0.044715) * (x * x))))


def _silu_half(d):
    hd = 0.25 * d
    return hd * (1.0 + jnp.tanh(hd))


def _dot(a, b):
    return jnp.dot(a, b, preferred_element_type=f32)


def _dot_nt(a, b):
    return lax.dot_general(a, b, (((1,), (1,)), ((), ())), preferred_element_type=f32)


def _lanesum(p):
    zp = p[:, 0:G]
    for j in range(1, p.shape[1] // G):
        zp = zp + p[:, j * G:(j + 1) * G]
    return zp


def _quad(a):
    r, c = a.shape[0] // 2, a.shape[1] // 2
    return [a[:r, :c], a[:r, c:], a[r:, :c], a[r:, c:]]


def _unquad(c):
    return jnp.concatenate([jnp.concatenate(c[:2], axis=1), jnp.concatenate(c[2:], axis=1)], axis=0)


def _lhs7(a, cast=True):
    c11, c12, c21, c22 = [x.astype(f32) for x in a]
    ops = [c11 + c22, c21 + c22, a[0], a[3], c11 + c12, c21 - c11, c12 - c22]
    return [x.astype(bf16) for x in ops] if cast else ops


def _rhs7(b, c=None, cast=True):
    c11, c12, c21, c22 = [x.astype(f32) for x in b] if c is None else c
    ops = [c11 + c22, b[0], c12 - c22, c21 - c11, b[3], c11 + c12, c21 + c22]
    return [x.astype(bf16) for x in ops] if cast else ops


def _strassen_gen(prod, out):
    m5 = prod(4)
    yield
    m3 = prod(2)
    yield
    m2 = prod(1)
    yield
    m4 = prod(3)
    yield
    m1 = prod(0)
    yield
    c11 = prod(6) + (m1 + (m4 - m5))
    yield
    c22 = prod(5) + (m1 + (m3 - m2))
    out.extend([c11, m3 + m5, m2 + m4, c22])
    yield


def _run(*gens):
    gens = list(gens)
    while gens:
        gens = [g for g in gens if next(g, 0) is None]


def _strassen(prod):
    out = []
    _run(_strassen_gen(prod, out))
    return out


def _kernel(x_hbm, wqkv_hbm, wo_hbm, wg_hbm, wu_hbm, wd_hbm, out_hbm,
            x_v, xn_u, xs_u, wq_v, wk_v, wv_v, wo_v, wg_v, wu_v, wd_v, out_v,
            a_acc, ma_acc, z_acc, rk_u, rm_u, rq_u, pq_v, wqt_u, wkt_u, pk0_u, zrow_v,
            sem, osem, consts):
    def xcopy(i):
        rows = pl.ds(X_OFFS[i], X_CHUNKS[i])
        return pltpu.make_async_copy(x_hbm.at[:, rows], x_v.at[:, rows], sem.at[8 + i])

    wk_cp = [pltpu.make_async_copy(wqkv_hbm.at[:, pl.ds(D + hh * HD, HD)], wk_v.at[hh], sem.at[7 * hh])
             for hh in range(2)]
    wq_cp = pltpu.make_async_copy(wqkv_hbm.at[:, pl.ds(0, D)], wq_v, sem.at[1])
    wv_cp = pltpu.make_async_copy(wqkv_hbm.at[:, pl.ds(2 * D, D)], wv_v, sem.at[2])
    wo_cp = pltpu.make_async_copy(wo_hbm, wo_v, sem.at[3])
    wg_cp = pltpu.make_async_copy(wg_hbm, wg_v, sem.at[4])
    wu_cp = pltpu.make_async_copy(wu_hbm, wu_v, sem.at[5])
    wd_cp = pltpu.make_async_copy(wd_hbm, wd_v, sem.at[6])

    def put(dst_u, pair0, val):
        dst_u[pl.ds(pair0, val.shape[0] // 2), :] = pltpu.bitcast(val, u32)

    def store_t(dst_u, w, p0=0):
        n = w.shape[1] // 2
        for c in range(dst_u.shape[0]):
            dst_u[c, pl.ds(p0, n), :] = pltpu.bitcast(w[c * G:(c + 1) * G, :].T, u32)

    def load_rows(src_u, blocks, cs=None):
        rows = []
        for p0, nh in blocks:
            blk = [src_u[c, pl.ds(p0, nh, stride=HP), :] for c in (cs or range(src_u.shape[0]))]
            rows.append(blk[0] if len(blk) == 1 else jnp.concatenate(blk, axis=1))
        return pltpu.bitcast(jnp.concatenate(rows, axis=0), bf16)

    def load_qorder(src_u):
        return load_rows(src_u, [(dp, H) for dp in range(HP)])

    def load_korder(src_u, groups=range(NG), cs=None):
        return load_rows(src_u, [(g * HG * HP + dp, HG) for g in groups for dp in range(HP)], cs)

    def rhs7_t(wt):
        b11, b21, b12, b22 = _quad(wt)
        return _rhs7([b11, b12, b21, b22])

    def raw_x(o, t, dt=f32):
        return jnp.concatenate([x_v.at[hf][pl.ds(o, t), :].astype(dt) for hf in range(2)], axis=0)

    def ln(o, t):
        x = raw_x(o, t)
        m = jnp.mean(x, axis=-1, keepdims=True)
        xc = x - m
        v = jnp.mean(xc * xc, axis=-1, keepdims=True)
        rstd = jnp.exp2(-0.5 * jnp.log2(v + 1e-5))
        return xc * rstd, m, rstd

    def ln_plain(o, t):
        xn, m, rstd = ln(o, t)
        for hf in range(2):
            put(xn_u.at[hf], o // 2, xn[hf * t:(hf + 1) * t].astype(bf16))
        return xn.astype(bf16), m, rstd

    def store_ops(o, ops):
        for i, op in enumerate(ops):
            put(xs_u.at[i], o // 2, op)
        return ops

    def load_op(i, pair0, t):
        return pltpu.bitcast(xs_u[i, pl.ds(pair0, t // 2), :], bf16)

    def load_xn(o, t):
        return jnp.concatenate([pltpu.bitcast(xn_u[hf, pl.ds(o // 2, t // 2), :], bf16) for hf in range(2)], axis=0)

    def inv_den(pq):
        t4 = _lanesum(pq * zrow_v[0:1, :])
        u = t4 + pltpu.roll(t4, 64, 1)
        even = (lax.broadcasted_iota(jnp.int32, u.shape, 1) & 1) == 0
        den = u + jnp.where(even, pltpu.roll(u, G - 1, 1), pltpu.roll(u, 1, 1)) + 1e-6
        return 1.0 / den

    def phase2(it, carry):
        base = pl.multiple_of(it * P, P)
        lx = [load_op(i, pl.multiple_of(it * (P // 2), P // 2), P) for i in range(7)]
        lx2 = [_lhs7(_quad(l)) for l in lx]

        lr = []
        for b, ts in enumerate(OUT_BLOCKS):
            u, r0 = divmod(sum(OUT_BLOCKS[:b]), TQ)
            ps = [pq_v[2 * it + u, hf][r0:r0 + ts] for hf in range(2)]
            iv = [inv_den(p) for p in ps]
            iv = [jnp.concatenate([v, v], axis=1) for v in iv]
            lr.append(_lhs7([ps[0][:, :HD] * iv[0], ps[0][:, HD:] * iv[0],
                             ps[1][:, :HD] * iv[1], ps[1][:, HD:] * iv[1]]))

        def wblocks(n, dt, z=0):
            rows = lambda k0: pl.ds(k0 if isinstance(z, int) else pl.multiple_of(z + k0, 16), HD)
            return [jnp.concatenate([wg_v[rows(k0), c].astype(dt), wu_v[rows(k0), c].astype(dt)], axis=1)
                    for k0 in (0, HD) for c in (pl.ds(n * G, G), pl.ds(HF + n * G, G))]

        def gate_up(n, out):
            r7 = _rhs7(wblocks(n, bf16), wblocks(n, f32))
            return _strassen_gen(lambda i: _dot(lx[i], r7[i]), out)

        def gate_up2(n, out):
            quad = lambda a, b: [a[:G], b[:G], a[G:], b[G:]]

            def outer(i):
                wide = quad(*[_rhs7(wblocks(m, f32, consts[1 + i]), cast=False)[i] for m in (n, n + 1)])
                raw = quad(*[wblocks(m, bf16)[0 if i == 1 else 3] for m in (n, n + 1)]) if i in (1, 4) else wide
                r2 = _rhs7(raw, wide)
                return _unquad(_strassen(lambda j: _dot(lx2[i][j], r2[j])))
            return _strassen_gen(outer, out)

        def hidden(cs):
            return [jnp.concatenate([_geglu2(c[:, o:o + G], c[:, o + G:o + 2 * G])
                                     for o in range(0, c.shape[1], 2 * G)], axis=1) for c in cs]

        md = [None] * 7

        def down(ns, hs):
            lh = _lhs7(hs, cast=False)
            blk = lambda dt: [jnp.concatenate([wd_v[pl.ds(k0 + n * G, G), pl.ds(n0, HD)].astype(dt) for n in ns], axis=0)
                              for k0 in (0, HF) for n0 in (0, HD)]
            rd = _rhs7(blk(bf16), blk(f32))
            for i in D_ORDER:
                if len(ns) % 2 and i == D_ORDER[-1]:
                    md[i] = jnp.concatenate([_dot(lh[i][r:r + P // 2].astype(bf16), rd[i]) for r in (0, P // 2)], axis=0)
                else:
                    d = _dot(lh[i].astype(bf16), rd[i])
                    md[i] = d if md[i] is None else d + md[i]
                yield

        c6, ca, cb, cc = [], [], [], []
        _run(gate_up(6, c6), gate_up2(0, ca))
        ha = hidden(ca)
        _run(gate_up2(2, cb), down((6, 0, 1), [jnp.concatenate(p, axis=1) for p in zip(hidden(c6), ha)]))
        _run(gate_up2(4, cc), down((2, 3), hidden(cb)))
        _run(down((4, 5), hidden(cc)))
        gts = [_silu_half(d) for d in _strassen(lambda i: md[i])]

        for b, ts in enumerate(OUT_BLOCKS):
            o = sum(OUT_BLOCKS[:b])
            ss = _strassen(lambda i: _dot(lr[b][i], pltpu.bitcast(rm_u[i], bf16)))
            for k in (1, 2, 0, 3):
                half, cs = k // 2, pl.ds((k % 2) * HD, HD)
                xr = x_v[half, pl.ds(pl.multiple_of(base + o, 16), ts), cs]
                y = (xr.astype(f32) + ss[k] * gts[k][o:o + ts]).astype(bf16)
                parts = LAST_SPLIT if (b == len(OUT_BLOCKS) - 1 and k == 3) else 1
                tp = ts // parts
                for p in range(parts):
                    rp = pl.ds(pl.multiple_of(base + o + p * tp, 16), tp)
                    out_v[half, rp, cs] = y[p * tp:(p + 1) * tp, :]
                    pltpu.make_async_copy(out_v.at[half, rp, cs], out_hbm.at[half, rp, cs], osem.at[0]).start()
        return carry

    def main(_, carry):
        ha, hb = pl.ds(0, HD), pl.ds(HD, HD)

        xcopy(0).wait()
        ln_plain(0, B0)
        wk_cp[0].wait()
        pk11 = _phi(_dot(load_xn(0, B0), wk_v[0])).astype(bf16)
        store_t(wkt_u, wk_v.at[0], 0)
        csum = jnp.sum(wk_v[0].astype(f32), axis=0, keepdims=True)
        xcopy(1).wait()
        y = _dot(raw_x(B0, B0, bf16), wk_v[0])
        _, m, rstd = ln_plain(B0, B0)
        pk21 = _phi((y - m * csum) * rstd).astype(bf16)
        pk0_u[0, pl.ds(0, HD // 2), :] = pltpu.bitcast(pk11.T, u32)
        pk = load_korder(pk0_u, (0, 1), (0,))
        a_acc[ha, :] = _dot(pk, load_xn(0, B0))
        z_acc[ha, :] = pk.astype(f32)
        wk_cp[1].wait()
        xcopy(2).wait()
        pk0_u[1, pl.ds(0, HD // 2), :] = pltpu.bitcast(pk21.T, u32)
        xn01 = jnp.concatenate([load_xn(0, B0), load_xn(B0, B0)], axis=0)
        store_t(pk0_u, _phi(_dot(xn01, wk_v[1])).astype(bf16), HD // 2)
        store_t(wkt_u, wk_v.at[1], HD // 2)
        xnb = ln_plain(2 * B0, B0)[0]
        pk = load_korder(pk0_u, (0, 1), (1,))
        a_acc[ha, :] += _dot(pk, load_xn(B0, B0))
        z_acc[ha, :] += pk.astype(f32)
        pkt = _phi(_dot_nt(load_korder(wkt_u), xnb))
        pk = load_korder(pk0_u, (2, 3))
        a_acc[hb, :] = _dot(pk, xn01)
        z_acc[hb, :] = _lanesum(pk.astype(f32))
        z_acc[...] += _lanesum(pkt)
        xcopy(3).wait()
        a_acc[...] += _dot(pkt.astype(bf16), load_xn(2 * B0, B0))
        pkt = _phi(_dot_nt(load_korder(wkt_u), ln_plain(3 * B0, B0)[0]))
        z_acc[...] += _lanesum(pkt)
        a_acc[...] += _dot(pkt.astype(bf16), load_xn(3 * B0, B0))

        def k_block(b, r7):
            xn = ln((b + 1) * G, G)[0]
            lx = store_ops((b + 1) * G, _lhs7(_quad(xn)))
            if r7 is None:
                p11, p21, p12, p22 = _quad(_phi(_dot_nt(load_korder(wkt_u), xn.astype(bf16))))
            else:
                p11, p12, p21, p22 = [_phi(c) for c in _strassen(lambda i: _dot_nt(r7[i], lx[i]))]
            z_acc[ha, :] += p11 + p21
            z_acc[hb, :] += p12 + p22
            return b, _lhs7([p11, p21, p12, p22])

        def a_blocks(blocks, idxs, first=False):
            for i in idxs:
                d = None if first else ma_acc[i]
                for b, lp in blocks:
                    p = _dot(lp[i], load_op(X_AS_RHS[i], (b + 1) * G // 2, G))
                    d = p if d is None else p + d
                ma_acc[i] = d

        def q_unit(u):
            lx = [load_op(i, u * TQ // 2, TQ) for i in range(7)]
            q = _strassen(lambda i: _dot_nt(lx[i], pltpu.bitcast(rq_u[i], bf16)))
            pq_v[u, 0] = _phi(jnp.concatenate(q[:2], axis=1))
            pq_v[u, 1] = _phi(jnp.concatenate(q[2:], axis=1))

        rk = lambda: [pltpu.bitcast(rk_u[i], bf16) for i in range(7)]
        l1 = k_block(1, None)
        r7 = rhs7_t(load_korder(wkt_u))
        for i in range(7):
            put(rk_u.at[i], 0, r7[i])
        l2 = k_block(2, r7)
        a_blocks([l1, l2], A_ORDER[:4], True)
        l3 = k_block(3, rk())
        xcopy(4).wait()
        wq_cp.wait()
        wv_cp.wait()
        wo_cp.wait()
        store_t(wqt_u, wq_v)
        for i, op in enumerate(rhs7_t(load_qorder(wqt_u))):
            put(rq_u.at[i], 0, op)
        a_blocks([l1, l2], A_ORDER[4:], True)
        l4 = k_block(4, rk())
        q_unit(1)
        l5 = k_block(5, rk())
        a_blocks([l3, l4], A_ORDER)
        l6 = k_block(6, rk())
        q_unit(2)
        a_blocks([l5, l6], A_ORDER)
        q_unit(3)
        a_acc[...] += _unquad(_strassen(lambda i: ma_acc[i]))

        zq = jnp.concatenate([z_acc[pl.ds(g * G + dp * DH, DH), :] for dp in range(HP) for g in range(NG)], axis=0)
        zrow_v[...] = jnp.broadcast_to(jnp.sum(zq.T, axis=0, keepdims=True), zrow_v.shape)

        row_head = (lax.broadcasted_iota(jnp.int32, (G, G), 0) % DH) // 2
        col_head = lax.broadcasted_iota(jnp.int32, (G, G), 1) // DH
        kvs = []
        for g in range(NG):
            sl = slice(g * G, (g + 1) * G)
            kv = _dot(a_acc[sl, :].astype(bf16), wv_v[:, sl])
            kvs.append(jnp.where(row_head == col_head, kv, 0.0).astype(bf16))
        for g in range(NG):
            mg = _dot(kvs[g], wo_v[g * G:(g + 1) * G, :])
            for i, op in enumerate(_rhs7(_quad(mg), cast=False)):
                for dp in range(HP // 2):
                    put(rm_u.at[i], dp * H + HP * g, op[dp * DH:(dp + 1) * DH, :].astype(bf16))
        store_ops(0, _lhs7(_quad(load_xn(0, R0))))
        q_unit(0)

        wg_cp.wait()
        wu_cp.wait()
        wd_cp.wait()
        lax.fori_loop(0, NIT, phase2, 0)
        return carry

    consts[0] = 1
    for i in range(7):
        consts[1 + i] = 0
    xcopy(0).start()
    wk_cp[0].start()
    xcopy(1).start()
    wk_cp[1].start()
    for i in range(2, len(X_CHUNKS)):
        xcopy(i).start()
    for cp in (wq_cp, wv_cp, wo_cp, wg_cp, wu_cp, wd_cp):
        cp.start()
    lax.fori_loop(0, consts[0], main, 0)
    pltpu.make_async_copy(out_v, out_hbm, osem.at[0]).wait()


@jax.jit
def pallas_recurrent_scan__linear_attn_block__geglu_ffn__prompt_kernel(
    A_x: jax.Array,
    A_wqkv: jax.Array,
    A_wo: jax.Array,
    B_x: jax.Array,
    B_w_gate: jax.Array,
    B_w_up: jax.Array,
    B_w_down: jax.Array,
):
    del B_x
    hbm = pl.BlockSpec(memory_space=pl.ANY)
    pairs = D // 2 + 2 * HP
    out = pl.pallas_call(
        _kernel,
        out_shape=jax.ShapeDtypeStruct((2, HS, D), bf16),
        in_specs=[hbm] * 6,
        out_specs=hbm,
        scratch_shapes=[
            pltpu.VMEM((2, HS, D), bf16),
            pltpu.VMEM((2, R0 // 2, D), u32),
            pltpu.VMEM((7, HS // 2, HD), u32),
            pltpu.VMEM((D, D), bf16),
            pltpu.VMEM((2, D, HD), bf16),
            pltpu.VMEM((D, D), bf16),
            pltpu.VMEM((D, D), bf16),
            pltpu.VMEM((D, F), bf16),
            pltpu.VMEM((D, F), bf16),
            pltpu.VMEM((F, D), bf16),
            pltpu.VMEM((2, HS, D), bf16),
            pltpu.VMEM((D, D), f32),
            pltpu.VMEM((7, HD, HD), f32),
            pltpu.VMEM((D, G), f32),
            pltpu.VMEM((7, HD // 2, HD), u32),
            pltpu.VMEM((7, HD // 2, HD), u32),
            pltpu.VMEM((7, HD // 2, HD), u32),
            pltpu.VMEM((HS // TQ, 2, TQ, D), f32),
            pltpu.VMEM((NG, pairs, G), u32),
            pltpu.VMEM((NG, pairs, G), u32),
            pltpu.VMEM((2, pairs, G), u32),
            pltpu.VMEM((8, D), f32),
            pltpu.SemaphoreType.DMA((8 + len(X_CHUNKS),)),
            pltpu.SemaphoreType.DMA((1,)),
            pltpu.SMEM((8,), jnp.int32),
        ],
        compiler_params=pltpu.CompilerParams(
            vmem_limit_bytes=100 * 1024 * 1024,
            disable_bounds_checks=True,
            disable_semaphore_checks=True,
        ),
    )(A_x.reshape(2, HS, D), A_wqkv, A_wo, B_w_gate, B_w_up, B_w_down)
    return out.reshape(1, S, D)
```

```python
import jax
import jax.numpy as jnp
from jax import lax
import jax.experimental.pallas as pl
import jax.experimental.pallas.tpu as pltpu

S, D, F = 2048, 512, 1792
H = 32
DH = D // H
G = 128
NG = D // G
HP = DH // 2
HG = G // DH
HS, HD, HF = S // 2, D // 2, F // 2

B0 = G // 2
BOTH = slice(None)
X_PIECES = ((BOTH, 0, B0), (BOTH, B0, B0), (0, G, G), (1, G, G), (BOTH, 2 * G, 2 * G), (BOTH, 4 * G, 4 * G))
NIT = 2
P = HS // NIT
TQ = P // 2
OUT_BLOCKS = (256, 128, 64, 64)
LAST_SPLIT = 2
X_AS_RHS = (0, 2, 6, 5, 3, 4, 1)
A_ORDER = (2, 4, 3, 0, 6, 5, 1)
D_ORDERS = ((4, 5, 3, 0, 1, 2, 6), (2, 5, 6, 0, 1, 4, 3), (2, 5, 3, 1, 4, 0, 6))
MERGE = ("ab" * 7, "aabb" + "ab" * 5, "abcabcabcbacabcabcabc")

f32 = jnp.float32
bf16 = jnp.bfloat16
u32 = jnp.uint32


def _phi(t):
    return jnp.where(t > 0, t + 1.0, jnp.exp(t)) + 1e-6


def _geglu2(x, up):
    c = 0.7978845608028654
    return (x * up) * (1.0 + jnp.tanh(x * (c + (c * 0.044715) * (x * x))))


def _silu_half(d):
    hd = 0.25 * d
    return hd * (1.0 + jnp.tanh(hd))


def _dot(a, b):
    return jnp.dot(a, b, preferred_element_type=f32)


def _dot_nt(a, b):
    return lax.dot_general(a, b, (((1,), (1,)), ((), ())), preferred_element_type=f32)


def _lanesum(p):
    zp = p[:, 0:G]
    for j in range(1, p.shape[1] // G):
        zp = zp + p[:, j * G:(j + 1) * G]
    return zp


def _quad(a):
    r, c = a.shape[0] // 2, a.shape[1] // 2
    return [a[:r, :c], a[:r, c:], a[r:, :c], a[r:, c:]]


def _unquad(c):
    return jnp.concatenate([jnp.concatenate(c[:2], axis=1), jnp.concatenate(c[2:], axis=1)], axis=0)


def _lhs7(a, cast=True):
    c11, c12, c21, c22 = [x.astype(f32) for x in a]
    ops = [c11 + c22, c21 + c22, a[0], a[3], c11 + c12, c21 - c11, c12 - c22]
    return [x.astype(bf16) for x in ops] if cast else ops


def _rhs7(b, c=None, cast=True):
    c11, c12, c21, c22 = [x.astype(f32) for x in b] if c is None else c
    ops = [c11 + c22, b[0], c12 - c22, c21 - c11, b[3], c11 + c12, c21 + c22]
    return [x.astype(bf16) for x in ops] if cast else ops


def _strassen_gen(prod, out, late=False):
    m5 = prod(4)
    yield
    m3 = prod(2)
    yield
    m2 = prod(1)
    yield
    m4 = prod(3)
    yield
    if late:
        c11 = prod(6) + (m4 - m5)
        yield
        m1 = prod(0)
        c11 = c11 + m1
    else:
        m1 = prod(0)
        yield
        c11 = prod(6) + (m1 + (m4 - m5))
    yield
    c22 = prod(5) + (m1 + (m3 - m2))
    out.extend([c11, m3 + m5, m2 + m4, c22])
    yield


def _run(order, *gens):
    for ch in order:
        next(gens["abc".index(ch)])


def _strassen(prod, late=False):
    out = []
    _run("a" * 7, _strassen_gen(prod, out, late))
    return out


def _kernel(x_hbm, wqkv_hbm, wo_hbm, wg_hbm, wu_hbm, wd_hbm, out_hbm,
            x_v, xn_u, xs_u, wq_v, wk_v, wv_v, wo_v, wg_v, wu_v, wd_v, out_v,
            a_acc, ma_acc, z_acc, rk_u, rm_u, rq_u, pq_v, wqt_u, wkt_u, pk0_u, zrow_v,
            sem, osem, consts):
    def xcopy(i):
        half, row0, rows = X_PIECES[i]
        idx = (half, pl.ds(row0, rows))
        return pltpu.make_async_copy(x_hbm.at[idx], x_v.at[idx], sem.at[8 + i])

    wk_cp = [pltpu.make_async_copy(wqkv_hbm.at[:, pl.ds(D + hh * HD, HD)], wk_v.at[hh], sem.at[7 * hh])
             for hh in range(2)]
    wq_cp = pltpu.make_async_copy(wqkv_hbm.at[:, pl.ds(0, D)], wq_v, sem.at[1])
    wv_cp = pltpu.make_async_copy(wqkv_hbm.at[:, pl.ds(2 * D, D)], wv_v, sem.at[2])
    wo_cp = pltpu.make_async_copy(wo_hbm, wo_v, sem.at[3])
    wg_cp = pltpu.make_async_copy(wg_hbm, wg_v, sem.at[4])
    wu_cp = pltpu.make_async_copy(wu_hbm, wu_v, sem.at[5])
    wd_cp = pltpu.make_async_copy(wd_hbm, wd_v, sem.at[6])

    def put(dst_u, pair0, val):
        dst_u[pl.ds(pair0, val.shape[0] // 2), :] = pltpu.bitcast(val, u32)

    def store_t(dst_u, w, p0=0):
        n = w.shape[1] // 2
        for c in range(dst_u.shape[0]):
            dst_u[c, pl.ds(p0, n), :] = pltpu.bitcast(w[c * G:(c + 1) * G, :].T, u32)

    def load_rows(src_u, blocks, cs=None):
        rows = []
        for p0, nh in blocks:
            blk = [src_u[c, pl.ds(p0, nh, stride=HP), :] for c in (cs or range(src_u.shape[0]))]
            rows.append(blk[0] if len(blk) == 1 else jnp.concatenate(blk, axis=1))
        return pltpu.bitcast(jnp.concatenate(rows, axis=0), bf16)

    def load_qorder(src_u):
        return load_rows(src_u, [(dp, H) for dp in range(HP)])

    def load_korder(src_u, groups=range(NG), cs=None):
        return load_rows(src_u, [(g * HG * HP + dp, HG) for g in groups for dp in range(HP)], cs)

    def rhs7_t(wt):
        b11, b21, b12, b22 = _quad(wt)
        return _rhs7([b11, b12, b21, b22])

    def raw_x(o, t, dt=f32):
        return jnp.concatenate([x_v.at[hf][pl.ds(o, t), :].astype(dt) for hf in range(2)], axis=0)

    def ln(o, t, hf=None):
        x = raw_x(o, t) if hf is None else x_v.at[hf][pl.ds(o, t), :].astype(f32)
        m = jnp.mean(x, axis=-1, keepdims=True)
        xc = x - m
        v = jnp.mean(xc * xc, axis=-1, keepdims=True)
        rstd = jnp.exp2(-0.5 * jnp.log2(v + 1e-5))
        return xc * rstd, m, rstd

    def ln_plain(o, t):
        xn, m, rstd = ln(o, t)
        for hf in range(2):
            put(xn_u.at[hf], o // 2, xn[hf * t:(hf + 1) * t].astype(bf16))
        return m, rstd

    def store_ops(o, ops):
        for i, op in enumerate(ops):
            put(xs_u.at[i], o // 2, op)
        return ops

    def load_op(i, pair0, t):
        return pltpu.bitcast(xs_u[i, pl.ds(pair0, t // 2), :], bf16)

    def load_xn(o, t):
        return jnp.concatenate([pltpu.bitcast(xn_u[hf, pl.ds(o // 2, t // 2), :], bf16) for hf in range(2)], axis=0)

    def inv_den(pq):
        t4 = _lanesum(pq * zrow_v[0:1, :])
        u = t4 + pltpu.roll(t4, 64, 1)
        even = (lax.broadcasted_iota(jnp.int32, u.shape, 1) & 1) == 0
        den = u + jnp.where(even, pltpu.roll(u, G - 1, 1), pltpu.roll(u, 1, 1)) + 1e-6
        return 1.0 / den

    def phase2(it, carry):
        base = pl.multiple_of(it * P, P)
        lx = [load_op(i, pl.multiple_of(it * (P // 2), P // 2), P) for i in range(7)]
        lx2 = [_lhs7(_quad(l)) for l in lx]

        lr = []
        for b, ts in enumerate(OUT_BLOCKS):
            u, r0 = divmod(sum(OUT_BLOCKS[:b]), TQ)
            ps = [pq_v[2 * it + u, hf][r0:r0 + ts] for hf in range(2)]
            iv = [inv_den(p) for p in ps]
            iv = [jnp.concatenate([v, v], axis=1) for v in iv]
            lr.append(_lhs7([ps[0][:, :HD] * iv[0], ps[0][:, HD:] * iv[0],
                             ps[1][:, :HD] * iv[1], ps[1][:, HD:] * iv[1]]))

        def wblocks(n, dt, z=0):
            rows = lambda k0: pl.ds(k0 if isinstance(z, int) else pl.multiple_of(z + k0, 16), HD)
            return [jnp.concatenate([wg_v[rows(k0), c].astype(dt), wu_v[rows(k0), c].astype(dt)], axis=1)
                    for k0 in (0, HD) for c in (pl.ds(n * G, G), pl.ds(HF + n * G, G))]

        def gate_up(n, out):
            r7 = _rhs7(wblocks(n, bf16), wblocks(n, f32))
            return _strassen_gen(lambda i: _dot(lx[i], r7[i]), out)

        def gate_up2(n, out):
            quad = lambda a, b: [a[:G], b[:G], a[G:], b[G:]]

            def outer(i):
                wide = quad(*[_rhs7(wblocks(m, f32, consts[1 + i]), cast=False)[i] for m in (n, n + 1)])
                raw = quad(*[wblocks(m, bf16)[0 if i == 1 else 3] for m in (n, n + 1)]) if i in (1, 4) else wide
                r2 = _rhs7(raw, wide)
                return _unquad(_strassen(lambda j: _dot(lx2[i][j], r2[j])))
            return _strassen_gen(outer, out)

        def hidden(cs):
            return [jnp.concatenate([_geglu2(c[:, o:o + G], c[:, o + G:o + 2 * G])
                                     for o in range(0, c.shape[1], 2 * G)], axis=1) for c in cs]

        md = [None] * 7

        def down(ns, hs, order):
            lh = _lhs7(hs, cast=False)
            blk = lambda dt: [jnp.concatenate([wd_v[pl.ds(k0 + n * G, G), pl.ds(n0, HD)].astype(dt) for n in ns], axis=0)
                              for k0 in (0, HF) for n0 in (0, HD)]
            rd = _rhs7(blk(bf16), blk(f32))
            for i in order:
                if len(ns) % 2 and i == order[-1]:
                    md[i] = jnp.concatenate([_dot(lh[i][r:r + P // 2].astype(bf16), rd[i]) for r in (0, P // 2)], axis=0)
                else:
                    d = _dot(lh[i].astype(bf16), rd[i])
                    md[i] = d if md[i] is None else d + md[i]
                yield

        def attn(b, out):
            return _strassen_gen(lambda i: _dot(lr[b][i], pltpu.bitcast(rm_u[i], bf16)), out, True)

        c6, ca, cb, cc, ss = [], [], [], [], []
        _run(MERGE[0], gate_up(6, c6), gate_up2(0, ca))
        ha = hidden(ca)
        h1 = [jnp.concatenate(p, axis=1) for p in zip(hidden(c6), ha)]
        _run(MERGE[1], gate_up2(2, cb), down((6, 0, 1), h1, D_ORDERS[0]))
        _run(MERGE[2], gate_up2(4, cc), down((2, 3), hidden(cb), D_ORDERS[1]), attn(0, ss))
        _run("a" * 7, down((4, 5), hidden(cc), D_ORDERS[2]))
        gts = [_silu_half(d) for d in _strassen(lambda i: md[i])]

        for b, ts in enumerate(OUT_BLOCKS):
            o = sum(OUT_BLOCKS[:b])
            if b:
                ss = []
                _run("a" * 7, attn(b, ss))
            for k in (1, 2, 0, 3):
                half, cs = k // 2, pl.ds((k % 2) * HD, HD)
                xr = x_v[half, pl.ds(pl.multiple_of(base + o, 16), ts), cs]
                y = (xr.astype(f32) + ss[k] * gts[k][o:o + ts]).astype(bf16)
                parts = LAST_SPLIT if (b == len(OUT_BLOCKS) - 1 and k == 3) else 1
                tp = ts // parts
                for p in range(parts):
                    rp = pl.ds(pl.multiple_of(base + o + p * tp, 16), tp)
                    out_v[half, rp, cs] = y[p * tp:(p + 1) * tp, :]
                    pltpu.make_async_copy(out_v.at[half, rp, cs], out_hbm.at[half, rp, cs], osem.at[0]).start()
        return carry

    def main(_, carry):
        ha, hb = pl.ds(0, HD), pl.ds(HD, HD)

        xcopy(0).wait()
        ln_plain(0, B0)
        wk_cp[0].wait()
        pk11 = _phi(_dot(load_xn(0, B0), wk_v[0])).astype(bf16)
        store_t(wkt_u, wk_v.at[0], 0)
        csum = jnp.sum(wk_v[0].astype(f32), axis=0, keepdims=True)
        xcopy(1).wait()
        y = _dot(raw_x(B0, B0, bf16), wk_v[0])
        m, rstd = ln_plain(B0, B0)
        pk21 = _phi((y - m * csum) * rstd).astype(bf16)
        pk0_u[0, pl.ds(0, HD // 2), :] = pltpu.bitcast(pk11.T, u32)
        pk = load_korder(pk0_u, (0, 1), (0,))
        a_acc[ha, :] = _dot(pk, load_xn(0, B0))
        z_acc[ha, :] = pk.astype(f32)
        wk_cp[1].wait()
        xcopy(2).wait()
        pk0_u[1, pl.ds(0, HD // 2), :] = pltpu.bitcast(pk21.T, u32)
        xn01 = lambda: jnp.concatenate([load_xn(0, B0), load_xn(B0, B0)], axis=0)
        store_t(pk0_u, _phi(_dot(xn01(), wk_v[1])).astype(bf16), HD // 2)
        store_t(wkt_u, wk_v.at[1], HD // 2)
        xt = ln(G, G, 0)[0]
        pk = load_korder(pk0_u, (0, 1), (1,))
        a_acc[ha, :] += _dot(pk, load_xn(B0, B0))
        z_acc[ha, :] += pk.astype(f32)
        pt = _phi(_dot_nt(load_korder(wkt_u), xt.astype(bf16)))
        xcopy(3).wait()
        xcopy(4).wait()
        pk = load_korder(pk0_u, (2, 3))
        a_acc[hb, :] = _dot(pk, xn01())
        z_acc[hb, :] = _lanesum(pk.astype(f32))
        xb = ln(G, G, 1)[0]
        pb = _phi(_dot_nt(load_korder(wkt_u), xb.astype(bf16)))
        store_ops(G, _lhs7([xt[:, :HD], xt[:, HD:], xb[:, :HD], xb[:, HD:]]))
        z_acc[...] += pt + pb
        l0 = (0, _lhs7([pt[:HD], pb[:HD], pt[HD:], pb[HD:]]))

        def k_block(b, r7):
            xn = ln((b + 1) * G, G)[0]
            lx = store_ops((b + 1) * G, _lhs7(_quad(xn)))
            if r7 is None:
                p11, p21, p12, p22 = _quad(_phi(_dot_nt(load_korder(wkt_u), xn.astype(bf16))))
            else:
                p11, p12, p21, p22 = [_phi(c) for c in _strassen(lambda i: _dot_nt(r7[i], lx[i]), True)]
            z_acc[ha, :] += p11 + p21
            z_acc[hb, :] += p12 + p22
            return b, _lhs7([p11, p21, p12, p22])

        def a_blocks(blocks, idxs, first=False):
            for i in idxs:
                d = None if first else ma_acc[i]
                for b, lp in blocks:
                    p = _dot(lp[i], load_op(X_AS_RHS[i], (b + 1) * G // 2, G))
                    d = p if d is None else p + d
                ma_acc[i] = d

        def q_unit(u):
            lx = [load_op(i, u * TQ // 2, TQ) for i in range(7)]
            q = _strassen(lambda i: _dot_nt(lx[i], pltpu.bitcast(rq_u[i], bf16)), True)
            pq_v[u, 0] = _phi(jnp.concatenate(q[:2], axis=1))
            pq_v[u, 1] = _phi(jnp.concatenate(q[2:], axis=1))

        rk = lambda: [pltpu.bitcast(rk_u[i], bf16) for i in range(7)]
        l1 = k_block(1, None)
        r7 = rhs7_t(load_korder(wkt_u))
        for i in range(7):
            put(rk_u.at[i], 0, r7[i])
        l2 = k_block(2, r7)
        a_blocks([l0, l1, l2], A_ORDER[:5], True)
        xcopy(5).wait()
        wq_cp.wait()
        wv_cp.wait()
        wo_cp.wait()
        store_t(wqt_u, wq_v)
        for i, op in enumerate(rhs7_t(load_qorder(wqt_u))):
            put(rq_u.at[i], 0, op)
        a_blocks([l0, l1, l2], A_ORDER[5:], True)
        l3 = k_block(3, rk())
        q_unit(1)
        l4 = k_block(4, rk())
        a_blocks([l3, l4], A_ORDER)
        l5 = k_block(5, rk())
        q_unit(2)
        l6 = k_block(6, rk())
        a_blocks([l5, l6], A_ORDER)
        q_unit(3)
        a_acc[...] += _unquad(_strassen(lambda i: ma_acc[i]))

        zq = jnp.concatenate([z_acc[pl.ds(g * G + dp * DH, DH), :] for dp in range(HP) for g in range(NG)], axis=0)
        zrow_v[...] = jnp.broadcast_to(jnp.sum(zq.T, axis=0, keepdims=True), zrow_v.shape)

        row_head = (lax.broadcasted_iota(jnp.int32, (G, G), 0) % DH) // 2
        col_head = lax.broadcasted_iota(jnp.int32, (G, G), 1) // DH
        kvs = []
        for g in range(NG):
            sl = slice(g * G, (g + 1) * G)
            kv = _dot(a_acc[sl, :].astype(bf16), wv_v[:, sl])
            kvs.append(jnp.where(row_head == col_head, kv, 0.0).astype(bf16))
        for g in range(NG):
            mg = _dot(kvs[g], wo_v[g * G:(g + 1) * G, :])
            for i, op in enumerate(_rhs7(_quad(mg), cast=False)):
                for dp in range(HP // 2):
                    put(rm_u.at[i], dp * H + HP * g, op[dp * DH:(dp + 1) * DH, :].astype(bf16))
        store_ops(0, _lhs7(_quad(load_xn(0, G))))
        q_unit(0)

        wg_cp.wait()
        wu_cp.wait()
        wd_cp.wait()
        lax.fori_loop(0, NIT, phase2, 0)
        return carry

    consts[0] = 1
    for i in range(7):
        consts[1 + i] = 0
    xcopy(0).start()
    wk_cp[0].start()
    xcopy(1).start()
    wk_cp[1].start()
    for i in range(2, len(X_PIECES)):
        xcopy(i).start()
    for cp in (wq_cp, wv_cp, wo_cp, wg_cp, wu_cp, wd_cp):
        cp.start()
    lax.fori_loop(0, consts[0], main, 0)
    pltpu.make_async_copy(out_v, out_hbm, osem.at[0]).wait()


@jax.jit
def pallas_recurrent_scan__linear_attn_block__geglu_ffn__prompt_kernel(
    A_x: jax.Array,
    A_wqkv: jax.Array,
    A_wo: jax.Array,
    B_x: jax.Array,
    B_w_gate: jax.Array,
    B_w_up: jax.Array,
    B_w_down: jax.Array,
):
    del B_x
    hbm = pl.BlockSpec(memory_space=pl.ANY)
    pairs = D // 2 + 2 * HP
    out = pl.pallas_call(
        _kernel,
        out_shape=jax.ShapeDtypeStruct((2, HS, D), bf16),
        in_specs=[hbm] * 6,
        out_specs=hbm,
        scratch_shapes=[
            pltpu.VMEM((2, HS, D), bf16),
            pltpu.VMEM((2, G // 2, D), u32),
            pltpu.VMEM((7, HS // 2, HD), u32),
            pltpu.VMEM((D, D), bf16),
            pltpu.VMEM((2, D, HD), bf16),
            pltpu.VMEM((D, D), bf16),
            pltpu.VMEM((D, D), bf16),
            pltpu.VMEM((D, F), bf16),
            pltpu.VMEM((D, F), bf16),
            pltpu.VMEM((F, D), bf16),
            pltpu.VMEM((2, HS, D), bf16),
            pltpu.VMEM((D, D), f32),
            pltpu.VMEM((7, HD, HD), f32),
            pltpu.VMEM((D, G), f32),
            pltpu.VMEM((7, HD // 2, HD), u32),
            pltpu.VMEM((7, HD // 2, HD), u32),
            pltpu.VMEM((7, HD // 2, HD), u32),
            pltpu.VMEM((HS // TQ, 2, TQ, D), f32),
            pltpu.VMEM((NG, pairs, G), u32),
            pltpu.VMEM((NG, pairs, G), u32),
            pltpu.VMEM((2, pairs, G), u32),
            pltpu.VMEM((8, D), f32),
            pltpu.SemaphoreType.DMA((8 + len(X_PIECES),)),
            pltpu.SemaphoreType.DMA((1,)),
            pltpu.SMEM((8,), jnp.int32),
        ],
        compiler_params=pltpu.CompilerParams(
            vmem_limit_bytes=100 * 1024 * 1024,
            disable_bounds_checks=True,
            disable_semaphore_checks=True,
        ),
    )(A_x.reshape(2, HS, D), A_wqkv, A_wo, B_w_gate, B_w_up, B_w_down)
    return out.reshape(1, S, D)
```

```python
import jax
import jax.numpy as jnp
from jax import lax
import jax.experimental.pallas as pl
import jax.experimental.pallas.tpu as pltpu

S, D, F = 2048, 512, 1792
H = 32
DH = D // H
G = 128
NG = D // G
HP = DH // 2
HG = G // DH
HS, HD, HF = S // 2, D // 2, F // 2

B0 = G // 2
BOTH = slice(None)
X_PIECES = ((BOTH, 0, B0), (BOTH, B0, B0), (0, G, G), (1, G, G), (BOTH, 2 * G, 2 * G), (BOTH, 4 * G, 4 * G))
NIT = 2
P = HS // NIT
TQ = P // 2
OUT_BLOCKS = (256, 128, 64, 64)
LAST_SPLIT = 2
X_AS_RHS = (0, 2, 6, 5, 3, 4, 1)
A_ORDERS = ((2, 4, 5, 0, 6, 3, 1), (2, 4, 3, 1, 6, 5, 0), (6, 4, 3, 0, 2, 5, 1))
D_ORDERS = ((4, 5, 3, 0, 1, 2, 6), (2, 5, 6, 0, 1, 4, 3), (2, 5, 3, 1, 4, 0, 6))
MERGE = ("ab" * 7, "aabb" + "ab" * 5, "abcabcabcbacabcabcabc")

f32 = jnp.float32
bf16 = jnp.bfloat16
u32 = jnp.uint32


def _phi(t):
    return jnp.where(t > 0, t + 1.0, jnp.exp(t)) + 1e-6


def _geglu2(x, up):
    c = 0.7978845608028654
    return (x * up) * (1.0 + jnp.tanh(x * (c + (c * 0.044715) * (x * x))))


def _silu_half(d):
    hd = 0.25 * d
    return hd * (1.0 + jnp.tanh(hd))


def _dot(a, b):
    return jnp.dot(a, b, preferred_element_type=f32)


def _dot_nt(a, b):
    return lax.dot_general(a, b, (((1,), (1,)), ((), ())), preferred_element_type=f32)


def _lanesum(p):
    zp = p[:, 0:G]
    for j in range(1, p.shape[1] // G):
        zp = zp + p[:, j * G:(j + 1) * G]
    return zp


def _quad(a):
    r, c = a.shape[0] // 2, a.shape[1] // 2
    return [a[:r, :c], a[:r, c:], a[r:, :c], a[r:, c:]]


def _unquad(c):
    return jnp.concatenate([jnp.concatenate(c[:2], axis=1), jnp.concatenate(c[2:], axis=1)], axis=0)


def _lhs7(a, cast=True):
    c11, c12, c21, c22 = [x.astype(f32) for x in a]
    ops = [c11 + c22, c21 + c22, a[0], a[3], c11 + c12, c21 - c11, c12 - c22]
    return [x.astype(bf16) for x in ops] if cast else ops


def _rhs7(b, c=None, cast=True):
    c11, c12, c21, c22 = [x.astype(f32) for x in b] if c is None else c
    ops = [c11 + c22, b[0], c12 - c22, c21 - c11, b[3], c11 + c12, c21 + c22]
    return [x.astype(bf16) for x in ops] if cast else ops


def _strassen_gen(prod, out, late=False):
    m5 = prod(4)
    yield
    m3 = prod(2)
    yield
    m2 = prod(1)
    yield
    m4 = prod(3)
    yield
    if late:
        c11 = prod(6) + (m4 - m5)
        yield
        m1 = prod(0)
        c11 = c11 + m1
    else:
        m1 = prod(0)
        yield
        c11 = prod(6) + (m1 + (m4 - m5))
    yield
    c22 = prod(5) + (m1 + (m3 - m2))
    out.extend([c11, m3 + m5, m2 + m4, c22])
    yield


def _run(order, *gens):
    for ch in order:
        next(gens["abc".index(ch)])


def _strassen(prod, late=False):
    out = []
    _run("a" * 7, _strassen_gen(prod, out, late))
    return out


def _kernel(x_hbm, wqkv_hbm, wo_hbm, wg_hbm, wu_hbm, wd_hbm, out_hbm,
            x_v, xn_u, xs_u, wq_v, wk_v, wv_v, wo_v, wg_v, wu_v, wd_v, out_v,
            a_acc, ma_acc, z_acc, rk_u, rm_u, rq_u, pq_v, wqt_u, wkt_u, pk0_u, zrow_v,
            sem, osem, consts):
    def xcopy(i):
        half, row0, rows = X_PIECES[i]
        idx = (half, pl.ds(row0, rows))
        return pltpu.make_async_copy(x_hbm.at[idx], x_v.at[idx], sem.at[8 + i])

    wk_cp = [pltpu.make_async_copy(wqkv_hbm.at[:, pl.ds(D + hh * HD, HD)], wk_v.at[hh], sem.at[7 * hh])
             for hh in range(2)]
    wq_cp = pltpu.make_async_copy(wqkv_hbm.at[:, pl.ds(0, D)], wq_v, sem.at[1])
    wv_cp = pltpu.make_async_copy(wqkv_hbm.at[:, pl.ds(2 * D, D)], wv_v, sem.at[2])
    wo_cp = pltpu.make_async_copy(wo_hbm, wo_v, sem.at[3])
    wg_cp = pltpu.make_async_copy(wg_hbm, wg_v, sem.at[4])
    wu_cp = pltpu.make_async_copy(wu_hbm, wu_v, sem.at[5])
    wd_cp = pltpu.make_async_copy(wd_hbm, wd_v, sem.at[6])

    def put(dst_u, pair0, val):
        dst_u[pl.ds(pair0, val.shape[0] // 2), :] = pltpu.bitcast(val, u32)

    def store_t(dst_u, w, p0=0):
        n = w.shape[1] // 2
        for c in range(dst_u.shape[0]):
            dst_u[c, pl.ds(p0, n), :] = pltpu.bitcast(w[c * G:(c + 1) * G, :].T, u32)

    def load_rows(src_u, blocks, cs=None):
        rows = []
        for p0, nh in blocks:
            blk = [src_u[c, pl.ds(p0, nh, stride=HP), :] for c in (cs or range(src_u.shape[0]))]
            rows.append(blk[0] if len(blk) == 1 else jnp.concatenate(blk, axis=1))
        return pltpu.bitcast(jnp.concatenate(rows, axis=0), bf16)

    def load_qorder(src_u):
        return load_rows(src_u, [(dp, H) for dp in range(HP)])

    def load_korder(src_u, groups=range(NG), cs=None):
        return load_rows(src_u, [(g * HG * HP + dp, HG) for g in groups for dp in range(HP)], cs)

    def rhs7_t(wt):
        b11, b21, b12, b22 = _quad(wt)
        return _rhs7([b11, b12, b21, b22])

    def raw_x(o, t, dt=f32):
        return jnp.concatenate([x_v.at[hf][pl.ds(o, t), :].astype(dt) for hf in range(2)], axis=0)

    def ln(o, t, hf=None):
        x = raw_x(o, t) if hf is None else x_v.at[hf][pl.ds(o, t), :].astype(f32)
        m = jnp.mean(x, axis=-1, keepdims=True)
        xc = x - m
        v = jnp.mean(xc * xc, axis=-1, keepdims=True)
        rstd = jnp.exp2(-0.5 * jnp.log2(v + 1e-5))
        return xc * rstd, m, rstd

    def ln_plain(o, t):
        xn, m, rstd = ln(o, t)
        for hf in range(2):
            put(xn_u.at[hf], o // 2, xn[hf * t:(hf + 1) * t].astype(bf16))
        return m, rstd

    def store_ops(o, ops):
        for i, op in enumerate(ops):
            put(xs_u.at[i], o // 2, op)
        return ops

    def load_op(i, pair0, t):
        return pltpu.bitcast(xs_u[i, pl.ds(pair0, t // 2), :], bf16)

    def load_xn(o, t):
        return jnp.concatenate([pltpu.bitcast(xn_u[hf, pl.ds(o // 2, t // 2), :], bf16) for hf in range(2)], axis=0)

    def inv_den(pq):
        t4 = _lanesum(pq * zrow_v[0:1, :])
        u = t4 + pltpu.roll(t4, 64, 1)
        even = (lax.broadcasted_iota(jnp.int32, u.shape, 1) & 1) == 0
        den = u + jnp.where(even, pltpu.roll(u, G - 1, 1), pltpu.roll(u, 1, 1)) + 1e-6
        return 1.0 / den

    def phase2(it, carry):
        base = pl.multiple_of(it * P, P)
        lx = [load_op(i, pl.multiple_of(it * (P // 2), P // 2), P) for i in range(7)]
        lx2 = [_lhs7(_quad(l)) for l in lx]

        lr = []
        for b, ts in enumerate(OUT_BLOCKS):
            u, r0 = divmod(sum(OUT_BLOCKS[:b]), TQ)
            ps = [pq_v[2 * it + u, hf][r0:r0 + ts] for hf in range(2)]
            iv = [inv_den(p) for p in ps]
            iv = [jnp.concatenate([v, v], axis=1) for v in iv]
            lr.append(_lhs7([ps[0][:, :HD] * iv[0], ps[0][:, HD:] * iv[0],
                             ps[1][:, :HD] * iv[1], ps[1][:, HD:] * iv[1]]))

        def wblocks(n, dt, z=0):
            rows = lambda k0: pl.ds(k0 if isinstance(z, int) else pl.multiple_of(z + k0, 16), HD)
            return [jnp.concatenate([wg_v[rows(k0), c].astype(dt), wu_v[rows(k0), c].astype(dt)], axis=1)
                    for k0 in (0, HD) for c in (pl.ds(n * G, G), pl.ds(HF + n * G, G))]

        def gate_up(n, out):
            r7 = _rhs7(wblocks(n, bf16), wblocks(n, f32))
            return _strassen_gen(lambda i: _dot(lx[i], r7[i]), out)

        def gate_up2(n, out):
            quad = lambda a, b: [a[:G], b[:G], a[G:], b[G:]]

            def outer(i):
                wide = quad(*[_rhs7(wblocks(m, f32, consts[1 + i]), cast=False)[i] for m in (n, n + 1)])
                raw = quad(*[wblocks(m, bf16)[0 if i == 1 else 3] for m in (n, n + 1)]) if i in (1, 4) else wide
                r2 = _rhs7(raw, wide)
                return _unquad(_strassen(lambda j: _dot(lx2[i][j], r2[j])))
            return _strassen_gen(outer, out)

        def hidden(cs):
            return [jnp.concatenate([_geglu2(c[:, o:o + G], c[:, o + G:o + 2 * G])
                                     for o in range(0, c.shape[1], 2 * G)], axis=1) for c in cs]

        md = [None] * 7

        def down(ns, hs, order):
            lh = _lhs7(hs, cast=False)
            blk = lambda dt: [jnp.concatenate([wd_v[pl.ds(k0 + n * G, G), pl.ds(n0, HD)].astype(dt) for n in ns], axis=0)
                              for k0 in (0, HF) for n0 in (0, HD)]
            rd = _rhs7(blk(bf16), blk(f32))
            for i in order:
                if len(ns) % 2 and i == order[-1]:
                    md[i] = jnp.concatenate([_dot(lh[i][r:r + P // 2].astype(bf16), rd[i]) for r in (0, P // 2)], axis=0)
                else:
                    d = _dot(lh[i].astype(bf16), rd[i])
                    md[i] = d if md[i] is None else d + md[i]
                yield

        def attn(b, out):
            return _strassen_gen(lambda i: _dot(lr[b][i], pltpu.bitcast(rm_u[i], bf16)), out, True)

        c6, ca, cb, cc, ss = [], [], [], [], []
        _run(MERGE[0], gate_up(6, c6), gate_up2(0, ca))
        ha = hidden(ca)
        h1 = [jnp.concatenate(p, axis=1) for p in zip(hidden(c6), ha)]
        _run(MERGE[1], gate_up2(2, cb), down((6, 0, 1), h1, D_ORDERS[0]))
        _run(MERGE[2], gate_up2(4, cc), down((2, 3), hidden(cb), D_ORDERS[1]), attn(0, ss))
        _run("a" * 7, down((4, 5), hidden(cc), D_ORDERS[2]))
        gts = [_silu_half(d) for d in _strassen(lambda i: md[i])]

        for b, ts in enumerate(OUT_BLOCKS):
            o = sum(OUT_BLOCKS[:b])
            if b:
                ss = []
                _run("a" * 7, attn(b, ss))
            for k in (1, 2, 0, 3):
                half, cs = k // 2, pl.ds((k % 2) * HD, HD)
                xr = x_v[half, pl.ds(pl.multiple_of(base + o, 16), ts), cs]
                y = (xr.astype(f32) + ss[k] * gts[k][o:o + ts]).astype(bf16)
                parts = LAST_SPLIT if (b == len(OUT_BLOCKS) - 1 and k == 3) else 1
                tp = ts // parts
                for p in range(parts):
                    rp = pl.ds(pl.multiple_of(base + o + p * tp, 16), tp)
                    out_v[half, rp, cs] = y[p * tp:(p + 1) * tp, :]
                    pltpu.make_async_copy(out_v.at[half, rp, cs], out_hbm.at[half, rp, cs], osem.at[0]).start()
        return carry

    def main(_, carry):
        ha, hb = pl.ds(0, HD), pl.ds(HD, HD)

        xcopy(0).wait()
        ln_plain(0, B0)
        wk_cp[0].wait()
        pk11 = _phi(_dot(load_xn(0, B0), wk_v[0])).astype(bf16)
        store_t(wkt_u, wk_v.at[0], 0)
        csum = jnp.sum(wk_v[0].astype(f32), axis=0, keepdims=True)
        xcopy(1).wait()
        y = _dot(raw_x(B0, B0, bf16), wk_v[0])
        m, rstd = ln_plain(B0, B0)
        pk21 = _phi((y - m * csum) * rstd).astype(bf16)
        pk0_u[0, pl.ds(0, HD // 2), :] = pltpu.bitcast(pk11.T, u32)
        pk = load_korder(pk0_u, (0, 1), (0,))
        a_acc[ha, :] = _dot(pk, load_xn(0, B0))
        z_acc[ha, :] = pk.astype(f32)
        wk_cp[1].wait()
        xcopy(2).wait()
        pk0_u[1, pl.ds(0, HD // 2), :] = pltpu.bitcast(pk21.T, u32)
        xn01 = lambda: jnp.concatenate([load_xn(0, B0), load_xn(B0, B0)], axis=0)
        store_t(pk0_u, _phi(_dot(xn01(), wk_v[1])).astype(bf16), HD // 2)
        store_t(wkt_u, wk_v.at[1], HD // 2)
        xt = ln(G, G, 0)[0]
        pk = load_korder(pk0_u, (0, 1), (1,))
        a_acc[ha, :] += _dot(pk, load_xn(B0, B0))
        z_acc[ha, :] += pk.astype(f32)
        pt = _phi(_dot_nt(load_korder(wkt_u), xt.astype(bf16)))
        xcopy(3).wait()
        xcopy(4).wait()
        pk = load_korder(pk0_u, (2, 3))
        a_acc[hb, :] = _dot(pk, xn01())
        z_acc[hb, :] = _lanesum(pk.astype(f32))
        xb = ln(G, G, 1)[0]
        pb = _phi(_dot_nt(load_korder(wkt_u), xb.astype(bf16)))
        store_ops(G, _lhs7([xt[:, :HD], xt[:, HD:], xb[:, :HD], xb[:, HD:]]))
        z_acc[...] += pt + pb
        l0 = (0, _lhs7([pt[:HD], pb[:HD], pt[HD:], pb[HD:]]))

        def k_block(b, r7):
            xn = ln((b + 1) * G, G)[0]
            lx = store_ops((b + 1) * G, _lhs7(_quad(xn)))
            if r7 is None:
                p11, p21, p12, p22 = _quad(_phi(_dot_nt(load_korder(wkt_u), xn.astype(bf16))))
            else:
                p11, p12, p21, p22 = [_phi(c) for c in _strassen(lambda i: _dot_nt(r7[i], lx[i]), True)]
            z_acc[ha, :] += p11 + p21
            z_acc[hb, :] += p12 + p22
            return b, _lhs7([p11, p21, p12, p22])

        def a_blocks(blocks, idxs, first=False):
            for i in idxs:
                d = None if first else ma_acc[i]
                for b, lp in blocks:
                    p = _dot(lp[i], load_op(X_AS_RHS[i], (b + 1) * G // 2, G))
                    d = p if d is None else p + d
                ma_acc[i] = d

        def q_unit(u):
            lx = [load_op(i, u * TQ // 2, TQ) for i in range(7)]
            q = _strassen(lambda i: _dot_nt(lx[i], pltpu.bitcast(rq_u[i], bf16)), True)
            pq_v[u, 0] = _phi(jnp.concatenate(q[:2], axis=1))
            pq_v[u, 1] = _phi(jnp.concatenate(q[2:], axis=1))

        rk = lambda: [pltpu.bitcast(rk_u[i], bf16) for i in range(7)]
        l1 = k_block(1, None)
        r7 = rhs7_t(load_korder(wkt_u))
        for i in range(7):
            put(rk_u.at[i], 0, r7[i])
        l2 = k_block(2, r7)
        a_blocks([l0, l1, l2], A_ORDERS[0][:5], True)
        xcopy(5).wait()
        wq_cp.wait()
        wv_cp.wait()
        wo_cp.wait()
        store_t(wqt_u, wq_v)
        for i, op in enumerate(rhs7_t(load_qorder(wqt_u))):
            put(rq_u.at[i], 0, op)
        a_blocks([l0, l1, l2], A_ORDERS[0][5:], True)
        l3 = k_block(3, rk())
        q_unit(1)
        l4 = k_block(4, rk())
        a_blocks([l3, l4], A_ORDERS[1])
        l5 = k_block(5, rk())
        q_unit(2)
        l6 = k_block(6, rk())
        a_blocks([l5, l6], A_ORDERS[2])
        q_unit(3)
        a_acc[...] += _unquad(_strassen(lambda i: ma_acc[i]))

        zq = jnp.concatenate([z_acc[pl.ds(g * G + dp * DH, DH), :] for dp in range(HP) for g in range(NG)], axis=0)
        zrow_v[...] = jnp.broadcast_to(jnp.sum(zq.T, axis=0, keepdims=True), zrow_v.shape)

        row_head = (lax.broadcasted_iota(jnp.int32, (G, G), 0) % DH) // 2
        col_head = lax.broadcasted_iota(jnp.int32, (G, G), 1) // DH
        kvs = []
        for g in range(NG):
            sl = slice(g * G, (g + 1) * G)
            kv = _dot(a_acc[sl, :].astype(bf16), wv_v[:, sl])
            kvs.append(jnp.where(row_head == col_head, kv, 0.0).astype(bf16))
        for g in range(NG):
            mg = _dot(kvs[g], wo_v[g * G:(g + 1) * G, :])
            for i, op in enumerate(_rhs7(_quad(mg), cast=False)):
                for dp in range(HP // 2):
                    put(rm_u.at[i], dp * H + HP * g, op[dp * DH:(dp + 1) * DH, :].astype(bf16))
        store_ops(0, _lhs7(_quad(load_xn(0, G))))
        q_unit(0)

        wg_cp.wait()
        wu_cp.wait()
        wd_cp.wait()
        lax.fori_loop(0, NIT, phase2, 0)
        return carry

    consts[0] = 1
    for i in range(7):
        consts[1 + i] = 0
    xcopy(0).start()
    wk_cp[0].start()
    xcopy(1).start()
    wk_cp[1].start()
    for i in range(2, len(X_PIECES)):
        xcopy(i).start()
    for cp in (wq_cp, wv_cp, wo_cp, wg_cp, wu_cp, wd_cp):
        cp.start()
    lax.fori_loop(0, consts[0], main, 0)
    pltpu.make_async_copy(out_v, out_hbm, osem.at[0]).wait()


@jax.jit
def pallas_recurrent_scan__linear_attn_block__geglu_ffn__prompt_kernel(
    A_x: jax.Array,
    A_wqkv: jax.Array,
    A_wo: jax.Array,
    B_x: jax.Array,
    B_w_gate: jax.Array,
    B_w_up: jax.Array,
    B_w_down: jax.Array,
):
    del B_x
    hbm = pl.BlockSpec(memory_space=pl.ANY)
    pairs = D // 2 + 2 * HP
    out = pl.pallas_call(
        _kernel,
        out_shape=jax.ShapeDtypeStruct((2, HS, D), bf16),
        in_specs=[hbm] * 6,
        out_specs=hbm,
        scratch_shapes=[
            pltpu.VMEM((2, HS, D), bf16),
            pltpu.VMEM((2, G // 2, D), u32),
            pltpu.VMEM((7, HS // 2, HD), u32),
            pltpu.VMEM((D, D), bf16),
            pltpu.VMEM((2, D, HD), bf16),
            pltpu.VMEM((D, D), bf16),
            pltpu.VMEM((D, D), bf16),
            pltpu.VMEM((D, F), bf16),
            pltpu.VMEM((D, F), bf16),
            pltpu.VMEM((F, D), bf16),
            pltpu.VMEM((2, HS, D), bf16),
            pltpu.VMEM((D, D), f32),
            pltpu.VMEM((7, HD, HD), f32),
            pltpu.VMEM((D, G), f32),
            pltpu.VMEM((7, HD // 2, HD), u32),
            pltpu.VMEM((7, HD // 2, HD), u32),
            pltpu.VMEM((7, HD // 2, HD), u32),
            pltpu.VMEM((HS // TQ, 2, TQ, D), f32),
            pltpu.VMEM((NG, pairs, G), u32),
            pltpu.VMEM((NG, pairs, G), u32),
            pltpu.VMEM((2, pairs, G), u32),
            pltpu.VMEM((8, D), f32),
            pltpu.SemaphoreType.DMA((8 + len(X_PIECES),)),
            pltpu.SemaphoreType.DMA((1,)),
            pltpu.SMEM((8,), jnp.int32),
        ],
        compiler_params=pltpu.CompilerParams(
            vmem_limit_bytes=100 * 1024 * 1024,
            disable_bounds_checks=True,
            disable_semaphore_checks=True,
        ),
    )(A_x.reshape(2, HS, D), A_wqkv, A_wo, B_w_gate, B_w_up, B_w_down)
    return out.reshape(1, S, D)
```

```python
import jax
import jax.numpy as jnp
from jax import lax
import jax.experimental.pallas as pl
import jax.experimental.pallas.tpu as pltpu

S, D, F = 2048, 512, 1792
H = 32
DH = D // H
G = 128
NG = D // G
HP = DH // 2
HS, HD, HF = S // 2, D // 2, F // 2

B0 = G // 2
BOTH = slice(None)
X_PIECES = ((BOTH, 0, B0), (BOTH, B0, B0), (0, G, G), (1, G, G), (BOTH, 2 * G, 2 * G), (BOTH, 4 * G, 4 * G))
NIT = 2
P = HS // NIT
TQ = P // 2
OUT_BLOCKS = (256, 128, 64, 64)
LAST_SPLIT = 2
X_AS_RHS = (0, 2, 6, 5, 3, 4, 1)
A_ORDERS = ((2, 4, 5, 0, 6, 3, 1), (0, 4, 6, 1, 3, 5, 2), (6, 4, 3, 0, 2, 5, 1))
D_ORDERS = ((4, 5, 3, 0, 1, 2, 6), (2, 5, 6, 4, 1, 0, 3), (2, 5, 3, 1, 4, 0, 6))
MERGE = ("ab" * 7, "aabb" + "ab" * 5, "abcabcabcbacabcabcabc")

f32 = jnp.float32
bf16 = jnp.bfloat16
u32 = jnp.uint32


def _phi(t):
    return jnp.where(t > 0, t + 1.0, jnp.exp(t)) + 1e-6


def _geglu2(x, up):
    c = 0.7978845608028654
    return (x * up) * (1.0 + jnp.tanh(x * (c + (c * 0.044715) * (x * x))))


def _silu_half(d):
    hd = 0.25 * d
    return hd * (1.0 + jnp.tanh(hd))


def _dot(a, b):
    return jnp.dot(a, b, preferred_element_type=f32)


def _dot_nt(a, b):
    return lax.dot_general(a, b, (((1,), (1,)), ((), ())), preferred_element_type=f32)


def _lanesum(p):
    zp = p[:, 0:G]
    for j in range(1, p.shape[1] // G):
        zp = zp + p[:, j * G:(j + 1) * G]
    return zp


def _quad(a):
    r, c = a.shape[0] // 2, a.shape[1] // 2
    return [a[:r, :c], a[:r, c:], a[r:, :c], a[r:, c:]]


def _unquad(c):
    return jnp.concatenate([jnp.concatenate(c[:2], axis=1), jnp.concatenate(c[2:], axis=1)], axis=0)


def _lhs7(a, cast=True):
    c11, c12, c21, c22 = [x.astype(f32) for x in a]
    ops = [c11 + c22, c21 + c22, a[0], a[3], c11 + c12, c21 - c11, c12 - c22]
    return [x.astype(bf16) for x in ops] if cast else ops


def _rhs7(b, c=None, cast=True):
    c11, c12, c21, c22 = [x.astype(f32) for x in b] if c is None else c
    ops = [c11 + c22, b[0], c12 - c22, c21 - c11, b[3], c11 + c12, c21 + c22]
    return [x.astype(bf16) for x in ops] if cast else ops


def _strassen_gen(prod, out, late=False):
    m5 = prod(4)
    yield
    m3 = prod(2)
    yield
    m2 = prod(1)
    yield
    m4 = prod(3)
    yield
    if late:
        c11 = prod(6) + (m4 - m5)
        yield
        m1 = prod(0)
        c11 = c11 + m1
    else:
        m1 = prod(0)
        yield
        c11 = prod(6) + (m1 + (m4 - m5))
    yield
    c22 = prod(5) + (m1 + (m3 - m2))
    out.extend([c11, m3 + m5, m2 + m4, c22])
    yield


def _run(order, *gens):
    for ch in order:
        next(gens["abc".index(ch)])


def _strassen(prod, late=False):
    out = []
    _run("a" * 7, _strassen_gen(prod, out, late))
    return out


def _kernel(x_hbm, wqkv_hbm, wo_hbm, wg_hbm, wu_hbm, wd_hbm, out_hbm,
            x_v, xn_u, xs_u, wq_v, wk_v, wv_v, wo_v, wg_v, wu_v, wd_v, out_v,
            a_acc, ma_acc, z_acc, rk_u, rm_u, rq_u, pq_v, wqt_u, wkt_u, pk0_u, zrow_v,
            sem, osem, consts):
    def xcopy(i):
        half, row0, rows = X_PIECES[i]
        idx = (half, pl.ds(row0, rows))
        return pltpu.make_async_copy(x_hbm.at[idx], x_v.at[idx], sem.at[8 + i])

    wk_cp = [pltpu.make_async_copy(wqkv_hbm.at[:, pl.ds(D + hh * HD, HD)], wk_v.at[hh], sem.at[7 * hh])
             for hh in range(2)]
    wq_cp = pltpu.make_async_copy(wqkv_hbm.at[:, pl.ds(0, D)], wq_v, sem.at[1])
    wv_cp = pltpu.make_async_copy(wqkv_hbm.at[:, pl.ds(2 * D, D)], wv_v, sem.at[2])
    wo_cp = pltpu.make_async_copy(wo_hbm, wo_v, sem.at[3])
    wg_cp = pltpu.make_async_copy(wg_hbm, wg_v, sem.at[4])
    wu_cp = pltpu.make_async_copy(wu_hbm, wu_v, sem.at[5])
    wd_cp = pltpu.make_async_copy(wd_hbm, wd_v, sem.at[6])

    def put(dst_u, pair0, val):
        dst_u[pl.ds(pair0, val.shape[0] // 2), :] = pltpu.bitcast(val, u32)

    def store_t(dst_u, w, p0=0):
        n = w.shape[1] // 2
        for c in range(dst_u.shape[0]):
            dst_u[c, pl.ds(p0, n), :] = pltpu.bitcast(w[c * G:(c + 1) * G, :].T, u32)

    def load_perm(src_u, hh=None, cs=None):
        h0, nh = (0, H) if hh is None else (hh * H // 2, H // 2)
        rows = []
        for dp in range(HP):
            blk = [src_u[c, pl.ds(h0 * HP + dp, nh, stride=HP), :] for c in (cs or range(src_u.shape[0]))]
            rows.append(blk[0] if len(blk) == 1 else jnp.concatenate(blk, axis=1))
        return pltpu.bitcast(jnp.concatenate(rows, axis=0), bf16)

    def rhs7_t(wt):
        b11, b21, b12, b22 = _quad(wt)
        return _rhs7([b11, b12, b21, b22])

    def raw_x(o, t, dt=f32):
        return jnp.concatenate([x_v.at[hf][pl.ds(o, t), :].astype(dt) for hf in range(2)], axis=0)

    def ln(o, t, hf=None):
        x = raw_x(o, t) if hf is None else x_v.at[hf][pl.ds(o, t), :].astype(f32)
        m = jnp.mean(x, axis=-1, keepdims=True)
        xc = x - m
        v = jnp.mean(xc * xc, axis=-1, keepdims=True)
        rstd = jnp.exp2(-0.5 * jnp.log2(v + 1e-5))
        return xc * rstd, m, rstd

    def ln_plain(o, t):
        xn, m, rstd = ln(o, t)
        for hf in range(2):
            put(xn_u.at[hf], o // 2, xn[hf * t:(hf + 1) * t].astype(bf16))
        return m, rstd

    def store_ops(o, ops):
        for i, op in enumerate(ops):
            put(xs_u.at[i], o // 2, op)
        return ops

    def load_op(i, pair0, t):
        return pltpu.bitcast(xs_u[i, pl.ds(pair0, t // 2), :], bf16)

    def load_xn(o, t):
        return jnp.concatenate([pltpu.bitcast(xn_u[hf, pl.ds(o // 2, t // 2), :], bf16) for hf in range(2)], axis=0)

    def inv_den(pq):
        t4 = _lanesum(pq * zrow_v[0:1, :])
        u = t4 + pltpu.roll(t4, 64, 1)
        even = (lax.broadcasted_iota(jnp.int32, u.shape, 1) & 1) == 0
        den = u + jnp.where(even, pltpu.roll(u, G - 1, 1), pltpu.roll(u, 1, 1)) + 1e-6
        return 1.0 / den

    def phase2(it, carry):
        base = pl.multiple_of(it * P, P)
        lx = [load_op(i, pl.multiple_of(it * (P // 2), P // 2), P) for i in range(7)]
        lx2 = [_lhs7(_quad(l)) for l in lx]

        lr = []
        for b, ts in enumerate(OUT_BLOCKS):
            u, r0 = divmod(sum(OUT_BLOCKS[:b]), TQ)
            ps = [pq_v[2 * it + u, hf][r0:r0 + ts] for hf in range(2)]
            iv = [inv_den(p) for p in ps]
            iv = [jnp.concatenate([v, v], axis=1) for v in iv]
            lr.append(_lhs7([ps[0][:, :HD] * iv[0], ps[0][:, HD:] * iv[0],
                             ps[1][:, :HD] * iv[1], ps[1][:, HD:] * iv[1]]))

        def wblocks(n, dt, z=0):
            rows = lambda k0: pl.ds(k0 if isinstance(z, int) else pl.multiple_of(z + k0, 16), HD)
            return [jnp.concatenate([wg_v[rows(k0), c].astype(dt), wu_v[rows(k0), c].astype(dt)], axis=1)
                    for k0 in (0, HD) for c in (pl.ds(n * G, G), pl.ds(HF + n * G, G))]

        def gate_up(n, out):
            r7 = _rhs7(wblocks(n, bf16), wblocks(n, f32))
            return _strassen_gen(lambda i: _dot(lx[i], r7[i]), out)

        def gate_up2(n, out):
            quad = lambda a, b: [a[:G], b[:G], a[G:], b[G:]]

            def outer(i):
                wide = quad(*[_rhs7(wblocks(m, f32, consts[1 + i]), cast=False)[i] for m in (n, n + 1)])
                raw = quad(*[wblocks(m, bf16)[0 if i == 1 else 3] for m in (n, n + 1)]) if i in (1, 4) else wide
                r2 = _rhs7(raw, wide)
                return _unquad(_strassen(lambda j: _dot(lx2[i][j], r2[j])))
            return _strassen_gen(outer, out)

        def hidden(cs):
            return [jnp.concatenate([_geglu2(c[:, o:o + G], c[:, o + G:o + 2 * G])
                                     for o in range(0, c.shape[1], 2 * G)], axis=1) for c in cs]

        md = [None] * 7

        def down(ns, hs, order):
            lh = _lhs7(hs, cast=False)
            blk = lambda dt: [jnp.concatenate([wd_v[pl.ds(k0 + n * G, G), pl.ds(n0, HD)].astype(dt) for n in ns], axis=0)
                              for k0 in (0, HF) for n0 in (0, HD)]
            rd = _rhs7(blk(bf16), blk(f32))
            for i in order:
                if len(ns) % 2 and i == order[-1]:
                    md[i] = jnp.concatenate([_dot(lh[i][r:r + P // 2].astype(bf16), rd[i]) for r in (0, P // 2)], axis=0)
                else:
                    d = _dot(lh[i].astype(bf16), rd[i])
                    md[i] = d if md[i] is None else d + md[i]
                yield

        def attn(b, out):
            return _strassen_gen(lambda i: _dot(lr[b][i], pltpu.bitcast(rm_u[i], bf16)), out, True)

        c6, ca, cb, cc, ss = [], [], [], [], []
        _run(MERGE[0], gate_up(6, c6), gate_up2(0, ca))
        ha = hidden(ca)
        h1 = [jnp.concatenate(p, axis=1) for p in zip(hidden(c6), ha)]
        _run(MERGE[1], gate_up2(2, cb), down((6, 0, 1), h1, D_ORDERS[0]))
        _run(MERGE[2], gate_up2(4, cc), down((2, 3), hidden(cb), D_ORDERS[1]), attn(0, ss))
        _run("a" * 7, down((4, 5), hidden(cc), D_ORDERS[2]))
        gts = [_silu_half(d) for d in _strassen(lambda i: md[i])]

        for b, ts in enumerate(OUT_BLOCKS):
            o = sum(OUT_BLOCKS[:b])
            if b:
                ss = []
                _run("a" * 7, attn(b, ss))
            for k in (1, 2, 0, 3):
                half, cs = k // 2, pl.ds((k % 2) * HD, HD)
                xr = x_v[half, pl.ds(pl.multiple_of(base + o, 16), ts), cs]
                y = (xr.astype(f32) + ss[k] * gts[k][o:o + ts]).astype(bf16)
                parts = LAST_SPLIT if (b == len(OUT_BLOCKS) - 1 and k == 3) else 1
                tp = ts // parts
                for p in range(parts):
                    rp = pl.ds(pl.multiple_of(base + o + p * tp, 16), tp)
                    out_v[half, rp, cs] = y[p * tp:(p + 1) * tp, :]
                    pltpu.make_async_copy(out_v.at[half, rp, cs], out_hbm.at[half, rp, cs], osem.at[0]).start()
        return carry

    def main(_, carry):
        def a_first(hh, cs, xn, add=False):
            pk = load_perm(pk0_u, hh, cs)
            a, z = _dot(pk, xn), _lanesum(pk.astype(f32))
            for dp in range(HP):
                rows, src = pl.ds((2 * dp + hh) * H, H), slice(dp * H, (dp + 1) * H)
                a_acc[rows, :] = a[src] + a_acc[rows, :] if add else a[src]
                z_acc[rows, :] = z[src] + z_acc[rows, :] if add else z[src]

        xcopy(0).wait()
        ln_plain(0, B0)
        wk_cp[0].wait()
        pk11 = _phi(_dot(load_xn(0, B0), wk_v[0])).astype(bf16)
        store_t(wkt_u, wk_v.at[0], 0)
        csum = jnp.sum(wk_v[0].astype(f32), axis=0, keepdims=True)
        xcopy(1).wait()
        y = _dot(raw_x(B0, B0, bf16), wk_v[0])
        m, rstd = ln_plain(B0, B0)
        pk21 = _phi((y - m * csum) * rstd).astype(bf16)
        pk0_u[0, pl.ds(0, HD // 2), :] = pltpu.bitcast(pk11.T, u32)
        a_first(0, (0,), load_xn(0, B0))
        wk_cp[1].wait()
        xcopy(2).wait()
        pk0_u[1, pl.ds(0, HD // 2), :] = pltpu.bitcast(pk21.T, u32)
        xn01 = lambda: jnp.concatenate([load_xn(0, B0), load_xn(B0, B0)], axis=0)
        store_t(pk0_u, _phi(_dot(xn01(), wk_v[1])).astype(bf16), HD // 2)
        store_t(wkt_u, wk_v.at[1], HD // 2)
        xt = ln(G, G, 0)[0]
        a_first(0, (1,), load_xn(B0, B0), True)
        pt = _phi(_dot_nt(load_perm(wkt_u), xt.astype(bf16)))
        xcopy(3).wait()
        xcopy(4).wait()
        a_first(1, None, xn01())
        xb = ln(G, G, 1)[0]
        pb = _phi(_dot_nt(load_perm(wkt_u), xb.astype(bf16)))
        store_ops(G, _lhs7([xt[:, :HD], xt[:, HD:], xb[:, :HD], xb[:, HD:]]))
        z_acc[...] += pt + pb
        l0 = (0, _lhs7([pt[:HD], pb[:HD], pt[HD:], pb[HD:]]))

        def k_block(b, r7):
            xn = ln((b + 1) * G, G)[0]
            lx = store_ops((b + 1) * G, _lhs7(_quad(xn)))
            if r7 is None:
                p11, p21, p12, p22 = _quad(_phi(_dot_nt(load_perm(wkt_u), xn.astype(bf16))))
            else:
                p11, p12, p21, p22 = [_phi(c) for c in _strassen(lambda i: _dot_nt(r7[i], lx[i]), True)]
            z_acc[:HD, :] += p11 + p21
            z_acc[HD:, :] += p12 + p22
            return b, _lhs7([p11, p21, p12, p22])

        def a_blocks(blocks, idxs, first=False):
            for i in idxs:
                d = None if first else ma_acc[i]
                for b, lp in blocks:
                    p = _dot(lp[i], load_op(X_AS_RHS[i], (b + 1) * G // 2, G))
                    d = p if d is None else p + d
                ma_acc[i] = d

        def q_unit(u):
            lx = [load_op(i, u * TQ // 2, TQ) for i in range(7)]
            q = _strassen(lambda i: _dot_nt(lx[i], pltpu.bitcast(rq_u[i], bf16)), True)
            pq_v[u, 0] = _phi(jnp.concatenate(q[:2], axis=1))
            pq_v[u, 1] = _phi(jnp.concatenate(q[2:], axis=1))

        rk = lambda: [pltpu.bitcast(rk_u[i], bf16) for i in range(7)]
        l1 = k_block(1, None)
        r7 = rhs7_t(load_perm(wkt_u))
        for i in range(7):
            put(rk_u.at[i], 0, r7[i])
        l2 = k_block(2, r7)
        a_blocks([l0, l1, l2], A_ORDERS[0][:5], True)
        xcopy(5).wait()
        wq_cp.wait()
        wv_cp.wait()
        wo_cp.wait()
        store_t(wqt_u, wq_v)
        for i, op in enumerate(rhs7_t(load_perm(wqt_u))):
            put(rq_u.at[i], 0, op)
        a_blocks([l0, l1, l2], A_ORDERS[0][5:], True)
        l3 = k_block(3, rk())
        q_unit(1)
        l4 = k_block(4, rk())
        a_blocks([l3, l4], A_ORDERS[1])
        l5 = k_block(5, rk())
        q_unit(2)
        l6 = k_block(6, rk())
        a_blocks([l5, l6], A_ORDERS[2])
        q_unit(3)
        a_acc[...] += _unquad(_strassen(lambda i: ma_acc[i]))

        zrow_v[...] = jnp.broadcast_to(jnp.sum(z_acc[...].T, axis=0, keepdims=True), zrow_v.shape)

        row_head = (lax.broadcasted_iota(jnp.int32, (G, G), 0) % DH) // 2
        col_head = lax.broadcasted_iota(jnp.int32, (G, G), 1) // DH
        kvs = []
        for g in range(NG):
            ag = jnp.concatenate([a_acc[pl.ds(2 * dp * H + DH * g, DH), :] for dp in range(HP)], axis=0)
            kv = _dot(ag.astype(bf16), wv_v[:, g * G:(g + 1) * G])
            kvs.append(jnp.where(row_head == col_head, kv, 0.0).astype(bf16))
        for g in range(NG):
            mg = _dot(kvs[g], wo_v[g * G:(g + 1) * G, :])
            for i, op in enumerate(_rhs7(_quad(mg), cast=False)):
                for dp in range(HP // 2):
                    put(rm_u.at[i], dp * H + HP * g, op[dp * DH:(dp + 1) * DH, :].astype(bf16))
        store_ops(0, _lhs7(_quad(load_xn(0, G))))
        q_unit(0)

        wg_cp.wait()
        wu_cp.wait()
        wd_cp.wait()
        lax.fori_loop(0, NIT, phase2, 0)
        return carry

    consts[0] = 1
    for i in range(7):
        consts[1 + i] = 0
    xcopy(0).start()
    wk_cp[0].start()
    xcopy(1).start()
    wk_cp[1].start()
    for i in range(2, len(X_PIECES)):
        xcopy(i).start()
    for cp in (wq_cp, wv_cp, wo_cp, wg_cp, wu_cp, wd_cp):
        cp.start()
    lax.fori_loop(0, consts[0], main, 0)
    pltpu.make_async_copy(out_v, out_hbm, osem.at[0]).wait()


@jax.jit
def pallas_recurrent_scan__linear_attn_block__geglu_ffn__prompt_kernel(
    A_x: jax.Array,
    A_wqkv: jax.Array,
    A_wo: jax.Array,
    B_x: jax.Array,
    B_w_gate: jax.Array,
    B_w_up: jax.Array,
    B_w_down: jax.Array,
):
    del B_x
    hbm = pl.BlockSpec(memory_space=pl.ANY)
    pairs = D // 2 + 2 * HP
    out = pl.pallas_call(
        _kernel,
        out_shape=jax.ShapeDtypeStruct((2, HS, D), bf16),
        in_specs=[hbm] * 6,
        out_specs=hbm,
        scratch_shapes=[
            pltpu.VMEM((2, HS, D), bf16),
            pltpu.VMEM((2, G // 2, D), u32),
            pltpu.VMEM((7, HS // 2, HD), u32),
            pltpu.VMEM((D, D), bf16),
            pltpu.VMEM((2, D, HD), bf16),
            pltpu.VMEM((D, D), bf16),
            pltpu.VMEM((D, D), bf16),
            pltpu.VMEM((D, F), bf16),
            pltpu.VMEM((D, F), bf16),
            pltpu.VMEM((F, D), bf16),
            pltpu.VMEM((2, HS, D), bf16),
            pltpu.VMEM((D, D), f32),
            pltpu.VMEM((7, HD, HD), f32),
            pltpu.VMEM((D, G), f32),
            pltpu.VMEM((7, HD // 2, HD), u32),
            pltpu.VMEM((7, HD // 2, HD), u32),
            pltpu.VMEM((7, HD // 2, HD), u32),
            pltpu.VMEM((HS // TQ, 2, TQ, D), f32),
            pltpu.VMEM((NG, pairs, G), u32),
            pltpu.VMEM((NG, pairs, G), u32),
            pltpu.VMEM((2, pairs, G), u32),
            pltpu.VMEM((8, D), f32),
            pltpu.SemaphoreType.DMA((8 + len(X_PIECES),)),
            pltpu.SemaphoreType.DMA((1,)),
            pltpu.SMEM((8,), jnp.int32),
        ],
        compiler_params=pltpu.CompilerParams(
            vmem_limit_bytes=100 * 1024 * 1024,
            disable_bounds_checks=True,
            disable_semaphore_checks=True,
        ),
    )(A_x.reshape(2, HS, D), A_wqkv, A_wo, B_w_gate, B_w_up, B_w_down)
    return out.reshape(1, S, D)
```
